```python
import jax
import jax.numpy as jnp

def _softmax(x, axis=-1):
    return jax.nn.softmax(x, axis=axis)

def _gelu(x):
    return jax.nn.gelu(x, approximate=True)

def _silu(x):
    return jax.nn.silu(x)

def _sigmoid(x):
    return jax.nn.sigmoid(x)

def _layernorm(x, axis=-1, eps=1e-05):
    m = jnp.mean(x, axis=axis, keepdims=True)
    v = jnp.var(x, axis=axis, keepdims=True)
    return (x - m) / jnp.sqrt(v + eps)

def _scatter_add(tgt, idx, src, axis=0):
    return tgt.at[idx].add(src)

def _segment_sum(src, seg, n):
    return jax.ops.segment_sum(src, seg, n)

class _Rng:

    def __init__(self, key):
        self._k = key

    def _next(self):
        self._k, sub = jax.random.split(self._k)
        return sub

    def normal(self, shape):
        return jax.random.normal(self._next(), shape, dtype=jnp.bfloat16)

    def randint(self, lo, hi, shape):
        return jax.random.randint(self._next(), shape, lo, hi, dtype=jnp.int32)

    def uniform(self, shape, lo=0.0, hi=1.0):
        return jax.random.uniform(self._next(), shape, jnp.bfloat16, lo, hi)

    def permutation(self, n):
        return jax.random.permutation(self._next(), n)
kernel_name = 'adaLN_cond__sliding_block_cached__moe_arch_mod__prompt'

def setup_inputs():
    _rng = _Rng(jax.random.key(int.from_bytes(__import__("os").urandom(4), "little")))
    _w = lambda a: (lambda t: t.astype(jnp.bfloat16) if jnp.issubdtype(t.dtype, jnp.floating) else t)(jnp.asarray(a))

    def _A_setup():
        B, Sq, D = (1, 2048, 1024)
        Hq, Hkv, Sk, Dh = (32, 4, 2048, 128)
        assert Hq % Hkv == 0, (Hq, Hkv)
        return {'x': _w((lambda *s: _rng.normal(s) * 0.05)(B, Sq, D)), 'k_cache': _w((lambda *s: _rng.normal(s) * 0.05)(B, Hkv, Sk, Dh)), 'v_cache': _w((lambda *s: _rng.normal(s) * 0.05)(B, Hkv, Sk, Dh)), 'wq': _w((lambda *s: _rng.normal(s) * 0.05)(D, Hq * Dh) * D ** (-0.5)), 'wo': _w((lambda *s: _rng.normal(s) * 0.05)(Hq * Dh, D) * (Hq * Dh) ** (-0.5))}
    _A_in = _A_setup()

    def _B_setup():
        B, S, D, F, C = (1, 2048, 1024, 3584, 1)
        return {'x': _w((lambda *s: _rng.normal(s) * 0.05)(B, S, D)), 'w_r': _w((lambda *s: _rng.normal(s) * 0.05)(D)), 'w_gate': _w((lambda *s: _rng.normal(s) * 0.05)(D, F)), 'w_up': _w((lambda *s: _rng.normal(s) * 0.05)(D, F)), 'w_down': _w((lambda *s: _rng.normal(s) * 0.05)(F, D))}
    _B_in = _B_setup()
    return {'A_x': _A_in['x'], 'A_k_cache': _A_in['k_cache'], 'A_v_cache': _A_in['v_cache'], 'A_wq': _A_in['wq'], 'A_wo': _A_in['wo'], 'B_x': _B_in['x'], 'B_w_r': _B_in['w_r'], 'B_w_gate': _B_in['w_gate'], 'B_w_up': _B_in['w_up'], 'B_w_down': _B_in['w_down'], 'c': _w((lambda *s: _rng.normal(s) * 0.05)(1, 1024)), 'w_mod': _w((lambda *s: _rng.normal(s) * 0.05)(1024, 6 * 1024) * 1024 ** (-0.5))}

def reference(A_x, A_k_cache, A_v_cache, A_wq, A_wo, B_x, B_w_r, B_w_gate, B_w_up, B_w_down, c, w_mod):

    def _A_ref(x, k_cache, v_cache, wq, wo):
        B, Sq, D = x.shape
        Hq, Dh = (32, 128)
        Hkv, Sk = (k_cache.shape[1], k_cache.shape[2])
        W = min(4096, max(256, Sk // 4))
        rep = Hq // Hkv
        q = (lambda x, *d: x.transpose(*d))((x @ wq).reshape(B, Sq, Hq, Dh), 0, 2, 1, 3)
        k = jnp.repeat(k_cache[:, :, Sk - W:, :], rep, axis=1)
        v = jnp.repeat(v_cache[:, :, Sk - W:, :], rep, axis=1)
        scores = jnp.einsum('bhqd,bhkd->bhqk', q, k) * Dh ** (-0.5)
        p = _softmax(scores, axis=-1)
        o = jnp.einsum('bhqk,bhkd->bhqd', p, v)
        return (lambda x, *d: x.transpose(*d))(o, 0, 2, 1, 3).reshape(B, Sq, Hq * Dh) @ wo

    def _B_ref(x, w_r, w_gate, w_up, w_down):
        B, S, D = x.shape
        C = 1
        r = x @ w_r
        idx = jnp.argsort(-r, axis=-1)[:, :C]
        idx_e = jnp.repeat(idx.reshape(B, C, 1), D, axis=2)
        x_sel = jnp.take_along_axis(x, idx_e, axis=1)
        g = _silu(x_sel @ w_gate)
        u = x_sel @ w_up
        y = g * u @ w_down
        r_sel = _sigmoid(jnp.take_along_axis(r, idx, axis=1))
        y = y * r_sel.reshape(B, C, 1)
        b_off = (jnp.arange(B) * S).reshape(B, 1)
        flat_idx = (idx + b_off).reshape(B * C)
        zero = (x * 0.0).reshape(B * S, D)
        upd = _scatter_add(zero, flat_idx, y.reshape(B * C, D), axis=0)
        return x + upd.reshape(B, S, D)
    x = A_x
    mod = (_silu(c) @ w_mod).reshape(c.shape[0], 6, 1, -1)
    sa, ca, ga, sb, cb, gb = (mod[:, 0].copy(), mod[:, 1].copy(), mod[:, 2].copy(), mod[:, 3].copy(), mod[:, 4].copy(), mod[:, 5].copy())
    h = _layernorm(x, axis=-1) * (1 + ca) + sa
    x = x + ga * _A_ref(h, A_k_cache, A_v_cache, A_wq, A_wo)
    h = _layernorm(x, axis=-1) * (1 + cb) + sb
    x = x + gb * _B_ref(h, B_w_r, B_w_gate, B_w_up, B_w_down)
    return x
```

```python
import contextlib

import jax
import jax.numpy as jnp
from jax import lax
import jax.experimental.pallas as pl
import jax.experimental.pallas.tpu as pltpu

BF = jnp.bfloat16
F32 = jnp.float32

S, D = 2048, 1024
HQ, HKV, DH = 32, 4, 128
REP = HQ // HKV
W = 512
FF = 3584
EPS = 1e-5
QSCALE = (DH ** -0.5) * 1.4426950408889634

TQ = 256
NT = S // TQ
NS = HQ
DELTA = 4
QB = 4
NSL = 16
RP = 16
NP = TQ // RP

H_OFF = 0
ROWS = 2 * TQ

_DEV = set()
_SCOPES = False


def _scope(name):
    return jax.named_scope(name) if _SCOPES else contextlib.nullcontext()


def _ln_mod(xf, scale1, shift):
    m = jnp.mean(xf, axis=-1, keepdims=True)
    xc = xf - m
    v = jnp.mean(xc * xc, axis=-1, keepdims=True)
    return xc * lax.rsqrt(v + EPS) * scale1 + shift


def _mult(v, m):
    return v if isinstance(v, int) else pl.multiple_of(v, m)


def _kernel(x_hbm, k_hbm, v_hbm, wq_hbm, wo_hbm, wr_hbm, wg_hbm, wu_hbm, wd_hbm, c_hbm, wmod_hbm,
            out_hbm,
            x_sc, row_sc, wq_sc, wo_sc, k_sc, v_sc, wmod_sc, wg_sc, wu_sc, wd_sc,
            c_sc, wr_sc, mod_sc, wrf_sc, q_sc, o_sc, aa_sc, xo_sc, sems):

    nsem = [0]

    def copy(src, dst):
        k = nsem[0]
        nsem[0] += 1
        return pltpu.make_async_copy(src, dst, sems.at[k])

    NMA = 2
    MCA = 2048 // NMA
    NMB = 4
    MCB = 4096 // NMB
    NWC = 8
    WC = 4096 // NWC
    HPC = HQ // NWC

    c_cp = copy(c_hbm, c_sc)
    wr_cp = copy(wr_hbm, wr_sc)
    x_cps = [copy(x_hbm.at[0, pl.ds(t * TQ, TQ), :], x_sc.at[pl.ds(t * TQ, TQ), :]) for t in range(NT)]
    wma_cps = [copy(wmod_hbm.at[:, pl.ds(t * MCA, MCA)], wmod_sc.at[:, pl.ds(t * MCA, MCA)]) for t in range(NMA)]
    wmb_cps = [copy(wmod_hbm.at[:, pl.ds(2048 + t * MCB, MCB)], wmod_sc.at[:, pl.ds(2048 + t * MCB, MCB)])
               for t in range(NMB)]
    wq_sem0 = nsem[0]
    wq_cps = [copy(wq_hbm.at[:, pl.ds(t * WC, WC)], wq_sc.at[:, pl.ds(t * WC, WC)]) for t in range(NWC)]
    wo_sem0 = nsem[0]
    wo_cps = [copy(wo_hbm.at[pl.ds(t * WC, WC), :], wo_sc.at[pl.ds(t * WC, WC), :]) for t in range(NWC)]
    k_cp = copy(k_hbm.at[0, :, pl.ds(k_hbm.shape[2] - W, W), :], k_sc)
    v_cp = copy(v_hbm.at[0, :, pl.ds(v_hbm.shape[2] - W, W), :], v_sc)
    ffn_cps = [copy(wg_hbm, wg_sc), copy(wu_hbm, wu_sc), copy(wd_hbm, wd_sc)]
    out_sem0 = nsem[0]
    nsem[0] += NT + 1

    def out_cp(t):
        r0 = _mult(t * TQ, TQ)
        return pltpu.make_async_copy(xo_sc.at[pl.ds(r0, TQ), :], out_hbm.at[0, pl.ds(r0, TQ), :],
                                     sems.at[out_sem0 + t])

    c_cp.start()
    x_cps[0].start()
    for cp in wma_cps:
        cp.start()
    wr_cp.start()
    wq_cps[0].start()
    k_cp.start()
    v_cp.start()
    wq_cps[1].start()
    wo_cps[0].start()
    x_cps[1].start()
    for t in range(1, NWC):
        if t + 1 < NWC:
            wq_cps[t + 1].start()
        wo_cps[t].start()
    for cp in wmb_cps:
        cp.start()
    for t in range(2, NT):
        x_cps[t].start()
    for cp in ffn_cps:
        cp.start()

    _sc = _scope("p0_prologue"); _sc.__enter__()
    c_cp.wait()
    cf = c_sc[...].astype(F32)
    sc16 = jnp.broadcast_to((cf * jax.nn.sigmoid(cf)).astype(BF), (16, D))

    def mod_chunk(c0, n):
        return jnp.dot(sc16, wmod_sc[:, c0:c0 + n], preferred_element_type=F32)[0:8, :]

    x_cps[0].wait()
    x0 = x_sc[0:TQ, :].astype(F32)
    m0 = jnp.mean(x0, axis=-1, keepdims=True)
    xc0 = x0 - m0
    xh0 = xc0 * lax.rsqrt(jnp.mean(xc0 * xc0, axis=-1, keepdims=True) + EPS)

    for t in range(NMA):
        wma_cps[t].wait()
        mod_sc[:, t * MCA:(t + 1) * MCA] = mod_chunk(t * MCA, MCA)
    row_sc[H_OFF:H_OFF + TQ, :] = (xh0 * (1.0 + mod_sc[0:1, D:2 * D]) + mod_sc[0:1, 0:D]).astype(BF)

    def q_proj(hslot, col, qslot):
        h = row_sc[pl.ds(_mult(H_OFF + hslot * TQ, TQ), TQ), :]
        q = jnp.dot(h, wq_sc[:, pl.ds(_mult(col, DH), DH)], preferred_element_type=F32)
        q_sc[qslot] = (q * QSCALE).astype(BF)

    wq_cps[0].wait()
    for m in range(DELTA):
        q_proj(0, m * DH, m % QB)
    _sc.__exit__(None, None, None)

    def a_piece(tile, k, hslot=None):
        r0 = _mult(tile * TQ + k * RP, RP)
        xf = x_sc[pl.ds(r0, RP), :].astype(F32)
        hh = _ln_mod(xf, 1.0 + mod_sc[0:1, D:2 * D], mod_sc[0:1, 0:D])
        hslot = jnp.bitwise_and(tile, 1) if hslot is None else hslot
        row_sc[pl.ds(_mult(H_OFF + hslot * TQ + k * RP, RP), RP), :] = hh.astype(BF)

    def h2_of(xp):
        return _ln_mod(xp.astype(F32), 1.0 + mod_sc[0:1, 4 * D:5 * D], mod_sc[0:1, 3 * D:4 * D])

    def e_piece(tile, k, best):
        bval, bidx = best
        r0 = _mult(tile * TQ + k * RP, RP)
        att = aa_sc[1, pl.ds(_mult(k * RP, RP), RP), :]
        xp = (x_sc[pl.ds(r0, RP), :].astype(F32) + mod_sc[0:1, 2 * D:3 * D] * att).astype(BF)
        xo_sc[pl.ds(S + r0, RP), :] = xp
        h2 = h2_of(xp)
        xo_sc[pl.ds(r0, RP), :] = (xp.astype(F32) + mod_sc[0:1, 5 * D:6 * D] * h2).astype(BF)
        r = jnp.sum(h2 * wrf_sc[0:1, :], axis=-1, keepdims=True)
        rows = r0 + lax.broadcasted_iota(jnp.int32, (RP, 1), 0)
        better = r > bval
        return jnp.where(better, r, bval), jnp.where(better, rows, bidx)

    def slot(j, g, wo_row, b_hslot, b_col, o_prev, d_mode, side):
        s = lax.dot_general(q_sc[j % QB], k_sc[g], (((1,), (1,)), ((), ())), preferred_element_type=F32)
        d = jnp.dot(o_prev, wo_sc[pl.ds(_mult(wo_row, DH), DH), :], preferred_element_type=F32)
        if d_mode == "acc":
            aa_sc[0] += d
        elif d_mode[0] == "finish":
            aa_sc[d_mode[1]] = aa_sc[0] + d
        else:
            aa_sc[0] = jnp.where(d_mode[1], 0.0, aa_sc[0]) + d
        for fn in side.get("early", ()):
            fn()
        mx = jnp.max(s, axis=-1, keepdims=True)
        pe = jnp.exp2(s - mx)
        l = jnp.sum(pe, axis=-1, keepdims=True)
        q_proj(b_hslot, b_col, (j + DELTA) % QB)
        o = jnp.dot(pe.astype(BF), v_sc[g], preferred_element_type=F32)
        rl = pl.reciprocal(l, approx=True)
        rl = rl * (2.0 - l * rl)
        o = (o * rl).astype(BF)
        for fn in side.get("late", ()):
            fn()
        return o

    def tile0_body(t, carry):
        @pl.when(t + 1 < NWC)
        def _():
            pltpu.make_async_copy(wq_hbm.at[:, pl.ds(0, WC)], wq_sc.at[:, pl.ds(0, WC)],
                                  sems.at[wq_sem0 + t + 1]).wait()
        pltpu.make_async_copy(wo_hbm.at[pl.ds(0, WC), :], wo_sc.at[pl.ds(0, WC), :], sems.at[wo_sem0 + t]).wait()

        @pl.when(t == 1)
        def _():
            x_cps[1].wait()
        o_prev = o_sc[...]
        tile_a = jnp.minimum(t, 1)
        last = t == NWC - 1
        col = t * WC
        b_col = jnp.where(last, 0, col + WC)
        b_hslot = last.astype(jnp.int32)
        g = lax.shift_right_logical(t, 1)
        for j in range(HPC):
            side = {}
            if j < 3:
                k = jnp.clip(3 * (t - 1) + j, 0, NP - 1)
                side = {"late": [lambda k=k: a_piece(tile_a, k)]}
            wo_row = jnp.maximum(col + (j - 1) * DH, 0)
            o_prev = slot(j, g, wo_row, b_hslot, b_col + j * DH, o_prev, "acc", side)
        o_sc[...] = o_prev
        return carry

    with _scope("p1_tile0"):
        k_cp.wait()
        v_cp.wait()
        o_sc[...] = jnp.zeros((TQ, DH), BF)
        aa_sc[0] = jnp.zeros((TQ, D), F32)
        lax.fori_loop(0, NWC, tile0_body, 0)

    _sc = _scope("p2_modrest"); _sc.__enter__()
    for cp in wmb_cps:
        cp.wait()
    wr_cp.wait()
    for t in range(2, NT):
        x_cps[t].wait()
    mod_sc[:, 2048:] = mod_chunk(2048, 4096)
    wrf_sc[...] = jnp.broadcast_to(wr_sc[...].astype(F32).reshape(1, D), (8, D))
    _sc.__exit__(None, None, None)

    IPT = NS // NSL
    assert IPT == 2 and HPC == DELTA and 2 * HPC == REP
    PPI = NP // IPT
    a_slot = {(k * (NSL - DELTA)) // PPI: k for k in range(PPI)}
    e_slot = {1 + (k * (NSL - 1)) // PPI: k for k in range(PPI)}

    def main_body(it, best):
        tile = lax.shift_right_logical(it, 1)
        part = jnp.bitwise_and(it, 1)
        first = part == 0
        base = part * (NSL * DH)
        nbase = NSL * DH - base
        hs_same = jnp.bitwise_and(tile, 1)
        hs_next = jnp.bitwise_and(tile + part, 1)
        best = list(best)
        o_prev = o_sc[...]
        for j in range(NSL):
            side = {"late": []}
            if j in a_slot and "noA" not in _DEV:
                side["late"].append(lambda k=a_slot[j]: a_piece(jnp.minimum(tile + 1, NT - 1), part * PPI + k))
            if j in e_slot and "noE" not in _DEV:
                def run_e(k=e_slot[j]):
                    best[:] = e_piece(tile - 1, part * PPI + k, best)
                side["late" if "eearly" not in _DEV else "early"] = side.get("late" if "eearly" not in _DEV else "early", []) + [run_e]
            mode = ("finish", 1 - part) if j == 0 else (("restart", first) if j == 1 else "acc")
            g = 2 * part + j // REP
            wo_row = base + (j - 1) * DH if j > 0 else (NS - 1) * DH - base
            if j + DELTA < NSL:
                b_hslot, b_col = hs_same, base + (j + DELTA) * DH
            else:
                b_hslot, b_col = hs_next, nbase + (j + DELTA - NSL) * DH
            o_prev = slot(j, g, wo_row, b_hslot, b_col, o_prev, mode, side)
        o_sc[...] = o_prev

        @pl.when(part == IPT - 1)
        def _():
            out_cp(tile - 1).start()
        return tuple(best)

    best = (jnp.full((RP, 1), -jnp.inf, F32), jnp.zeros((RP, 1), jnp.int32))
    with _scope("p3_loop"):
        best = lax.fori_loop(IPT, NT * IPT, main_body, best)

    _sc = _scope("p4_lastE"); _sc.__enter__()
    aa_sc[1] = aa_sc[0] + jnp.dot(o_sc[...], wo_sc[(NS - 1) * DH:NS * DH, :], preferred_element_type=F32)
    for k in range(NP):
        best = e_piece(NT - 1, k, best)
    out_cp(NT - 1).start()
    _sc.__exit__(None, None, None)

    _sc = _scope("p5_ffn"); _sc.__enter__()
    bval, bidx = best
    gmax = jnp.max(bval, axis=0, keepdims=True)
    idx = jnp.min(jnp.where(bval == gmax, bidx, S))
    r0 = pl.multiple_of((idx // RP) * RP, RP)
    xp = xo_sc[pl.ds(S + r0, RP), :]
    h2 = h2_of(xp)
    r = jnp.sum(h2 * wrf_sc[0:1, :], axis=-1, keepdims=True)
    for cp in ffn_cps:
        cp.wait()
    h2b = h2.astype(BF)
    gate = jnp.dot(h2b, wg_sc[...], preferred_element_type=F32)
    up = jnp.dot(h2b, wu_sc[...], preferred_element_type=F32)
    act = (gate * jax.nn.sigmoid(gate) * up).astype(BF)
    y = jnp.dot(act, wd_sc[...], preferred_element_type=F32) * jax.nn.sigmoid(r)
    rows = r0 + lax.broadcasted_iota(jnp.int32, (RP, 1), 0)
    upd = jnp.where(rows == idx, y, 0.0)
    fixed = (xp.astype(F32) + mod_sc[0:1, 5 * D:6 * D] * (h2 + upd)).astype(BF)
    _sc.__exit__(None, None, None)
    _sc = _scope("p6_out"); _sc.__enter__()
    for t in range(NT):
        out_cp(t).wait()
    row_sc[H_OFF:H_OFF + RP, :] = fixed
    fix_cp = pltpu.make_async_copy(row_sc.at[pl.ds(H_OFF, RP), :], out_hbm.at[0, pl.ds(r0, RP), :],
                                   sems.at[out_sem0 + NT])
    fix_cp.start()
    fix_cp.wait()
    _sc.__exit__(None, None, None)


_NSEM = 2 + NT + 2 + 4 + 8 + 8 + 2 + 3 + NT + 1


@jax.jit
def pallas_adaLN_cond__sliding_block_cached__moe_arch_mod__prompt_kernel(
    A_x: jax.Array,
    A_k_cache: jax.Array,
    A_v_cache: jax.Array,
    A_wq: jax.Array,
    A_wo: jax.Array,
    B_x: jax.Array,
    B_w_r: jax.Array,
    B_w_gate: jax.Array,
    B_w_up: jax.Array,
    B_w_down: jax.Array,
    c: jax.Array,
    w_mod: jax.Array,
):
    del B_x
    any_spec = pl.BlockSpec(memory_space=pl.ANY)
    scratch = [
        pltpu.VMEM((S, D), BF),
        pltpu.VMEM((ROWS, D), BF),
        pltpu.VMEM((D, HQ * DH), BF),
        pltpu.VMEM((HQ * DH, D), BF),
        pltpu.VMEM((HKV, W, DH), BF),
        pltpu.VMEM((HKV, W, DH), BF),
        pltpu.VMEM((D, 6 * D), BF),
        pltpu.VMEM((D, FF), BF),
        pltpu.VMEM((D, FF), BF),
        pltpu.VMEM((FF, D), BF),
        pltpu.VMEM((1, D), BF),
        pltpu.VMEM((D,), BF),
        pltpu.VMEM((8, 6 * D), F32),
        pltpu.VMEM((8, D), F32),
        pltpu.VMEM((QB, TQ, DH), BF),
        pltpu.VMEM((TQ, DH), BF),
        pltpu.VMEM((2, TQ, D), F32),
        pltpu.VMEM((2 * S, D), BF),
        pltpu.SemaphoreType.DMA((_NSEM,)),
    ]
    return pl.pallas_call(
        _kernel,
        out_shape=jax.ShapeDtypeStruct(A_x.shape, A_x.dtype),
        in_specs=[any_spec] * 11,
        out_specs=any_spec,
        scratch_shapes=scratch,
        compiler_params=pltpu.CompilerParams(vmem_limit_bytes=100 * 1024 * 1024),
    )(A_x, A_k_cache, A_v_cache, A_wq, A_wo, B_w_r, B_w_gate, B_w_up, B_w_down, c, w_mod)
```

```python
import contextlib

import jax
import jax.numpy as jnp
from jax import lax
import jax.experimental.pallas as pl
import jax.experimental.pallas.tpu as pltpu

BF = jnp.bfloat16
F32 = jnp.float32

S, D = 2048, 1024
HQ, HKV, DH = 32, 4, 128
REP = HQ // HKV
W = 512
FF = 3584
EPS = 1e-5
QSCALE = (DH ** -0.5) * 1.4426950408889634

TQ = 256
NT = S // TQ
NS = HQ
DELTA = 4
QB = 4
NSL = 16
DK0 = 4
DK = 4
RP = 16
NP = TQ // RP

H_OFF = 0
ROWS = 2 * TQ + S

_DEV = set()
_SCOPES = False


def _scope(name):
    return jax.named_scope(name) if _SCOPES else contextlib.nullcontext()


def _ln_mod(xf, scale1, shift):
    m = jnp.mean(xf, axis=-1, keepdims=True)
    xc = xf - m
    v = jnp.mean(xc * xc, axis=-1, keepdims=True)
    return xc * lax.rsqrt(v + EPS) * scale1 + shift


def _mult(v, m):
    return v if isinstance(v, int) else pl.multiple_of(v, m)


def _kernel(x_hbm, k_hbm, v_hbm, wq_hbm, wo_hbm, wr_hbm, wg_hbm, wu_hbm, wd_hbm, c_hbm, wmod_hbm,
            out_hbm,
            x_sc, row_sc, wq_sc, wo_sc, k_sc, v_sc, wmod_sc, wg_sc, wu_sc, wd_sc,
            c_sc, wr_sc, mod_sc, wrf_sc, q_sc, o_sc, acc_sc, att_sc, xo_sc, ep_sc, sems):

    nsem = [0]

    def copy(src, dst):
        k = nsem[0]
        nsem[0] += 1
        return pltpu.make_async_copy(src, dst, sems.at[k])

    NMA = 2
    MCA = 2048 // NMA
    NMB = 4
    MCB = 4096 // NMB
    NWC = 8
    WC = 4096 // NWC
    HPC = HQ // NWC

    c_cp = copy(c_hbm, c_sc)
    wr_cp = copy(wr_hbm, wr_sc)
    x_cps = [copy(x_hbm.at[0, pl.ds(t * TQ, TQ), :], x_sc.at[pl.ds(t * TQ, TQ), :]) for t in range(NT)]
    wma_cps = [copy(wmod_hbm.at[:, pl.ds(t * MCA, MCA)], wmod_sc.at[:, pl.ds(t * MCA, MCA)]) for t in range(NMA)]
    wmb_cps = [copy(wmod_hbm.at[:, pl.ds(2048 + t * MCB, MCB)], wmod_sc.at[:, pl.ds(2048 + t * MCB, MCB)])
               for t in range(NMB)]
    wq_sem0 = nsem[0]
    wq_cps = [copy(wq_hbm.at[:, pl.ds(t * WC, WC)], wq_sc.at[:, pl.ds(t * WC, WC)]) for t in range(NWC)]
    wo_sem0 = nsem[0]
    wo_cps = [copy(wo_hbm.at[pl.ds(t * WC, WC), :], wo_sc.at[pl.ds(t * WC, WC), :]) for t in range(NWC)]
    k_cp = copy(k_hbm.at[0, :, pl.ds(k_hbm.shape[2] - W, W), :], k_sc)
    v_cp = copy(v_hbm.at[0, :, pl.ds(v_hbm.shape[2] - W, W), :], v_sc)
    ffn_cps = [copy(wg_hbm, wg_sc), copy(wu_hbm, wu_sc), copy(wd_hbm, wd_sc)]
    out_sem0 = nsem[0]
    nsem[0] += NT + 1

    def out_cp(t):
        r0 = _mult(t * TQ, TQ)
        src_sc, src_off = (row_sc, 2 * TQ) if "pinE" in _DEV else (xo_sc, S)
        return pltpu.make_async_copy(src_sc.at[pl.ds(src_off + r0, TQ), :], out_hbm.at[0, pl.ds(r0, TQ), :],
                                     sems.at[out_sem0 + t])

    c_cp.start()
    x_cps[0].start()
    for cp in wma_cps:
        cp.start()
    wr_cp.start()
    wq_cps[0].start()
    k_cp.start()
    v_cp.start()
    wq_cps[1].start()
    wo_cps[0].start()
    x_cps[1].start()
    for t in range(1, NWC):
        if t + 1 < NWC:
            wq_cps[t + 1].start()
        wo_cps[t].start()
    for cp in wmb_cps:
        cp.start()
    for t in range(2, NT):
        x_cps[t].start()
    for cp in ffn_cps:
        cp.start()

    _sc = _scope("p0_prologue"); _sc.__enter__()
    c_cp.wait()
    cf = c_sc[...].astype(F32)
    sc16 = jnp.broadcast_to((cf * jax.nn.sigmoid(cf)).astype(BF), (16, D))

    def mod_chunk(c0, n):
        return jnp.dot(sc16, wmod_sc[:, c0:c0 + n], preferred_element_type=F32)[0:8, :]

    x_cps[0].wait()
    x0 = x_sc[0:TQ, :].astype(F32)
    m0 = jnp.mean(x0, axis=-1, keepdims=True)
    xc0 = x0 - m0
    xh0 = xc0 * lax.rsqrt(jnp.mean(xc0 * xc0, axis=-1, keepdims=True) + EPS)

    for t in range(NMA):
        wma_cps[t].wait()
        mod_sc[:, t * MCA:(t + 1) * MCA] = mod_chunk(t * MCA, MCA)
    row_sc[H_OFF:H_OFF + TQ, :] = (xh0 * (1.0 + mod_sc[0:1, D:2 * D]) + mod_sc[0:1, 0:D]).astype(BF)

    def q_proj(hslot, col, qslot):
        h = row_sc[pl.ds(_mult(H_OFF + hslot * TQ, TQ), TQ), :]
        q = jnp.dot(h, wq_sc[:, pl.ds(_mult(col, DH), DH)], preferred_element_type=F32)
        q_sc[qslot] = (q * QSCALE).astype(BF)

    wq_cps[0].wait()
    for m in range(DELTA):
        q_proj(0, m * DH, m % QB)
    _sc.__exit__(None, None, None)

    def a_piece(tile, k, hslot=None):
        r0 = _mult(tile * TQ + k * RP, RP)
        xf = x_sc[pl.ds(r0, RP), :].astype(F32)
        hh = _ln_mod(xf, 1.0 + mod_sc[0:1, D:2 * D], mod_sc[0:1, 0:D])
        hslot = jnp.bitwise_and(tile, 1) if hslot is None else hslot
        row_sc[pl.ds(_mult(H_OFF + hslot * TQ + k * RP, RP), RP), :] = hh.astype(BF)

    def h2_of(xp):
        return _ln_mod(xp.astype(F32), 1.0 + mod_sc[0:1, 4 * D:5 * D], mod_sc[0:1, 3 * D:4 * D])

    out_ref_sc, out_off = (row_sc, 2 * TQ) if "pinE" in _DEV else (xo_sc, S)

    def e_piece(tile, k, best):
        bval, bidx = best
        r0 = _mult(tile * TQ + k * RP, RP)
        att = att_sc[1, pl.ds(_mult(k * RP, RP), RP), :]
        xp = (x_sc[pl.ds(r0, RP), :].astype(F32) + mod_sc[0:1, 2 * D:3 * D] * att).astype(BF)
        xo_sc[pl.ds(r0, RP), :] = xp
        xf = xp.astype(F32)
        xc = xf - jnp.mean(xf, axis=-1, keepdims=True)
        rstd = lax.rsqrt(jnp.mean(xc * xc, axis=-1, keepdims=True) + EPS)
        out = (xf + ep_sc[1:2, :]) + (xc * rstd) * ep_sc[0:1, :]
        out_ref_sc[pl.ds(out_off + r0, RP), :] = out.astype(BF)
        r = jnp.sum(xc * ep_sc[2:3, :], axis=-1, keepdims=True) * rstd + ep_sc[3:4, 0:1]
        rows = r0 + lax.broadcasted_iota(jnp.int32, (RP, 1), 0)
        better = r > bval
        return jnp.where(better, r, bval), jnp.where(better, rows, bidx)

    def slot(j, g, wo_row, b_hslot, b_col, d_mode, side, dk):
        s = lax.dot_general(q_sc[j % QB], k_sc[g], (((1,), (1,)), ((), ())), preferred_element_type=F32)
        if j % dk == 0:
            d = jnp.dot(o_sc[:, 0:dk * DH], wo_sc[pl.ds(_mult(wo_row, DH), dk * DH), :], preferred_element_type=F32)
        if j % dk != 0:
            pass
        elif d_mode == "acc":
            acc_sc[...] += d
        elif d_mode[0] == "finish":
            t = acc_sc[...] + d
            att_sc[d_mode[1]] = t
            acc_sc[...] = t
        else:
            acc_sc[...] = jnp.where(d_mode[1], 0.0, acc_sc[...]) + d
        for fn in side.get("early", ()):
            fn()
        mx = jnp.max(s, axis=-1, keepdims=True)
        pe = jnp.exp2(s - mx)
        l = jnp.sum(pe, axis=-1, keepdims=True)
        q_proj(b_hslot, b_col, (j + DELTA) % QB)
        o = jnp.dot(pe.astype(BF), v_sc[g], preferred_element_type=F32)
        rl = pl.reciprocal(l, approx=True)
        rl = rl * (2.0 - l * rl)
        o_sc[:, (j % dk) * DH:(j % dk + 1) * DH] = (o * rl).astype(BF)
        for fn in side.get("late", ()):
            fn()

    def tile0_body(t, carry):
        @pl.when(t + 1 < NWC)
        def _():
            pltpu.make_async_copy(wq_hbm.at[:, pl.ds(0, WC)], wq_sc.at[:, pl.ds(0, WC)],
                                  sems.at[wq_sem0 + t + 1]).wait()
        pltpu.make_async_copy(wo_hbm.at[pl.ds(0, WC), :], wo_sc.at[pl.ds(0, WC), :], sems.at[wo_sem0 + t]).wait()

        @pl.when(t == 1)
        def _():
            x_cps[1].wait()
        tile_a = jnp.minimum(t, 1)
        last = t == NWC - 1
        col = t * WC
        b_col = jnp.where(last, 0, col + WC)
        b_hslot = last.astype(jnp.int32)
        g = lax.shift_right_logical(t, 1)
        for j in range(HPC):
            side = {}
            if j < 3:
                k = jnp.clip(3 * (t - 1) + j, 0, NP - 1)
                side = {"late": [lambda k=k: a_piece(tile_a, k)]}
            wo_row = jnp.maximum(col + (j - DK0) * DH, 0)
            slot(j, g, wo_row, b_hslot, b_col + j * DH, "acc", side, DK0)
        return carry

    with _scope("p1_tile0"):
        k_cp.wait()
        v_cp.wait()
        o_sc[...] = jnp.zeros((TQ, DK * DH), BF)
        acc_sc[...] = jnp.zeros((TQ, D), F32)
        lax.fori_loop(0, NWC, tile0_body, 0)
        if DK > DK0:
            o_sc[:, (DK - DK0) * DH:DK * DH] = o_sc[:, 0:DK0 * DH]
            o_sc[:, 0:(DK - DK0) * DH] = jnp.zeros((TQ, (DK - DK0) * DH), BF)

    _sc = _scope("p2_modrest"); _sc.__enter__()
    for cp in wmb_cps:
        cp.wait()
    wr_cp.wait()
    for t in range(2, NT):
        x_cps[t].wait()
    mod_sc[:, 2048:] = mod_chunk(2048, 4096)
    wrf_sc[...] = jnp.broadcast_to(wr_sc[...].astype(F32).reshape(1, D), (8, D))
    cb1 = 1.0 + mod_sc[0:1, 4 * D:5 * D]
    ep_sc[0:1, :] = mod_sc[0:1, 5 * D:6 * D] * cb1
    ep_sc[1:2, :] = mod_sc[0:1, 5 * D:6 * D] * mod_sc[0:1, 3 * D:4 * D]
    ep_sc[2:3, :] = cb1 * wrf_sc[0:1, :]
    ep_sc[3:4, :] = jnp.broadcast_to(
        jnp.sum(mod_sc[0:1, 3 * D:4 * D] * wrf_sc[0:1, :], axis=-1, keepdims=True), (1, D))
    _sc.__exit__(None, None, None)

    IPT = NS // NSL
    assert IPT == 2 and HPC == DELTA and 2 * HPC == REP
    PPI = NP // IPT
    a_slot = {(k * (NSL - DELTA)) // PPI: k for k in range(PPI)}
    e_slot = {1 + (k * (NSL - 1)) // PPI: k for k in range(PPI)}

    def main_body(it, best):
        tile = lax.shift_right_logical(it, 1)
        part = jnp.bitwise_and(it, 1)
        first = part == 0
        base = part * (NSL * DH)
        nbase = NSL * DH - base
        hs_same = jnp.bitwise_and(tile, 1)
        hs_next = jnp.bitwise_and(tile + part, 1)
        best = list(best)
        for j in range(NSL):
            side = {"late": []}
            if j in a_slot and "noA" not in _DEV:
                side["late"].append(lambda k=a_slot[j]: a_piece(jnp.minimum(tile + 1, NT - 1), part * PPI + k))
            if j in e_slot and "noE" not in _DEV:
                def run_e(k=e_slot[j]):
                    best[:] = e_piece(tile - 1, part * PPI + k, best)
                side["late" if "eearly" not in _DEV else "early"] = side.get("late" if "eearly" not in _DEV else "early", []) + [run_e]
            mode = ("finish", 1 - part) if j == 0 else (("restart", first) if j == DK else "acc")
            g = 2 * part + j // REP
            wo_row = base + (j - DK) * DH if j > 0 else (NS - DK) * DH - base
            if j + DELTA < NSL:
                b_hslot, b_col = hs_same, base + (j + DELTA) * DH
            else:
                b_hslot, b_col = hs_next, nbase + (j + DELTA - NSL) * DH
            slot(j, g, wo_row, b_hslot, b_col, mode, side, DK)

        @pl.when(part == IPT - 1)
        def _():
            out_cp(tile - 1).start()
        return tuple(best)

    best = (jnp.full((RP, 1), -jnp.inf, F32), jnp.zeros((RP, 1), jnp.int32))
    with _scope("p3_loop"):
        best = lax.fori_loop(IPT, NT * IPT, main_body, best)

    _sc = _scope("p4_lastE"); _sc.__enter__()
    att_sc[1] = acc_sc[...] + jnp.dot(o_sc[...], wo_sc[(NS - DK) * DH:NS * DH, :], preferred_element_type=F32)
    for k in range(NP):
        best = e_piece(NT - 1, k, best)
    out_cp(NT - 1).start()
    _sc.__exit__(None, None, None)

    _sc = _scope("p5_ffn"); _sc.__enter__()
    bval, bidx = best
    gmax = jnp.max(bval, axis=0, keepdims=True)
    idx = jnp.min(jnp.where(bval == gmax, bidx, S))
    r0 = pl.multiple_of((idx // RP) * RP, RP)
    xp = xo_sc[pl.ds(r0, RP), :]
    h2 = h2_of(xp)
    r = jnp.sum(h2 * wrf_sc[0:1, :], axis=-1, keepdims=True)
    for cp in ffn_cps:
        cp.wait()
    h2b = h2.astype(BF)
    gate = jnp.dot(h2b, wg_sc[...], preferred_element_type=F32)
    up = jnp.dot(h2b, wu_sc[...], preferred_element_type=F32)
    act = (gate * jax.nn.sigmoid(gate) * up).astype(BF)
    y = jnp.dot(act, wd_sc[...], preferred_element_type=F32) * jax.nn.sigmoid(r)
    rows = r0 + lax.broadcasted_iota(jnp.int32, (RP, 1), 0)
    upd = jnp.where(rows == idx, y, 0.0)
    fixed = (xp.astype(F32) + mod_sc[0:1, 5 * D:6 * D] * (h2 + upd)).astype(BF)
    _sc.__exit__(None, None, None)
    _sc = _scope("p6_out"); _sc.__enter__()
    for t in range(NT):
        out_cp(t).wait()
    row_sc[H_OFF:H_OFF + RP, :] = fixed
    fix_cp = pltpu.make_async_copy(row_sc.at[pl.ds(H_OFF, RP), :], out_hbm.at[0, pl.ds(r0, RP), :],
                                   sems.at[out_sem0 + NT])
    fix_cp.start()
    fix_cp.wait()
    _sc.__exit__(None, None, None)


_NSEM = 2 + NT + 2 + 4 + 8 + 8 + 2 + 3 + NT + 1


@jax.jit
def pallas_adaLN_cond__sliding_block_cached__moe_arch_mod__prompt_kernel(
    A_x: jax.Array,
    A_k_cache: jax.Array,
    A_v_cache: jax.Array,
    A_wq: jax.Array,
    A_wo: jax.Array,
    B_x: jax.Array,
    B_w_r: jax.Array,
    B_w_gate: jax.Array,
    B_w_up: jax.Array,
    B_w_down: jax.Array,
    c: jax.Array,
    w_mod: jax.Array,
):
    del B_x
    any_spec = pl.BlockSpec(memory_space=pl.ANY)
    scratch = [
        pltpu.VMEM((S, D), BF),
        pltpu.VMEM((ROWS, D), BF),
        pltpu.VMEM((D, HQ * DH), BF),
        pltpu.VMEM((HQ * DH, D), BF),
        pltpu.VMEM((HKV, W, DH), BF),
        pltpu.VMEM((HKV, W, DH), BF),
        pltpu.VMEM((D, 6 * D), BF),
        pltpu.VMEM((D, FF), BF),
        pltpu.VMEM((D, FF), BF),
        pltpu.VMEM((FF, D), BF),
        pltpu.VMEM((1, D), BF),
        pltpu.VMEM((D,), BF),
        pltpu.VMEM((8, 6 * D), F32),
        pltpu.VMEM((8, D), F32),
        pltpu.VMEM((QB, TQ, DH), BF),
        pltpu.VMEM((TQ, DK * DH), BF),
        pltpu.VMEM((TQ, D), F32),
        pltpu.VMEM((2, TQ, D), F32),
        pltpu.VMEM((2 * S, D), BF),
        pltpu.VMEM((8, D), F32),
        pltpu.SemaphoreType.DMA((_NSEM,)),
    ]
    return pl.pallas_call(
        _kernel,
        out_shape=jax.ShapeDtypeStruct(A_x.shape, A_x.dtype),
        in_specs=[any_spec] * 11,
        out_specs=any_spec,
        scratch_shapes=scratch,
        compiler_params=pltpu.CompilerParams(vmem_limit_bytes=100 * 1024 * 1024),
    )(A_x, A_k_cache, A_v_cache, A_wq, A_wo, B_w_r, B_w_gate, B_w_up, B_w_down, c, w_mod)
```

```python
import contextlib

import jax
import jax.numpy as jnp
from jax import lax
import jax.experimental.pallas as pl
import jax.experimental.pallas.tpu as pltpu

BF = jnp.bfloat16
F32 = jnp.float32

S, D = 2048, 1024
HQ, HKV, DH = 32, 4, 128
REP = HQ // HKV
W = 512
FF = 3584
EPS = 1e-5
QSCALE = (DH ** -0.5) * 1.4426950408889634

TQ = 256
NT = S // TQ
NS = HQ
DELTA = 4
QB = 4
NSL = 16
DK0 = 4
DK = 4
PAD = 128
APAD = 0
RP = 16
NP = TQ // RP

H_OFF = 0
ROWS = 2 * TQ + S

_DEV = set()
_SCOPES = False


def _scope(name):
    return jax.named_scope(name) if _SCOPES else contextlib.nullcontext()


def _ln_mod(xf, scale1, shift):
    m = jnp.mean(xf, axis=-1, keepdims=True)
    xc = xf - m
    v = jnp.mean(xc * xc, axis=-1, keepdims=True)
    return xc * lax.rsqrt(v + EPS) * scale1 + shift


def _mult(v, m):
    return v if isinstance(v, int) else pl.multiple_of(v, m)


def _kernel(x_hbm, k_hbm, v_hbm, wq_hbm, wo_hbm, wr_hbm, wg_hbm, wu_hbm, wd_hbm, c_hbm, wmod_hbm,
            out_hbm,
            x_sc, row_sc, wq_sc, wo_sc, k_sc, v_sc, wmod_sc, wg_sc, wu_sc, wd_sc,
            c_sc, wr_sc, mod_sc, wrf_sc, q_sc, o_sc, acc_sc, att_sc, xo_sc, ep_sc, sems):

    nsem = [0]

    def copy(src, dst):
        k = nsem[0]
        nsem[0] += 1
        return pltpu.make_async_copy(src, dst, sems.at[k])

    NMA = 4
    MCA = 2048 // NMA
    NMB = 4
    MCB = 4096 // NMB
    NWC = 8
    WC = 4096 // NWC
    HPC = HQ // NWC

    c_cp = copy(c_hbm, c_sc)
    wr_cp = copy(wr_hbm, wr_sc)
    x_sem0 = nsem[0]
    x_cps = [copy(x_hbm.at[0, pl.ds(t * TQ, TQ), :], x_sc.at[pl.ds(t * TQ, TQ), :]) for t in range(NT)]
    wma_cps = [copy(wmod_hbm.at[:, pl.ds(t * MCA, MCA)], wmod_sc.at[:, pl.ds(t * MCA, MCA)]) for t in range(NMA)]
    wmb_cps = [copy(wmod_hbm.at[:, pl.ds(2048 + t * MCB, MCB)], wmod_sc.at[:, pl.ds(2048 + t * MCB, MCB)])
               for t in range(NMB)]
    wq_sem0 = nsem[0]
    wq_cps = [copy(wq_hbm.at[:, pl.ds(t * WC, WC)], wq_sc.at[:, pl.ds(t * WC, WC)]) for t in range(NWC)]
    wo_sem0 = nsem[0]
    wo_cps = [copy(wo_hbm.at[pl.ds(t * WC, WC), :], wo_sc.at[pl.ds(t * WC, WC), pl.ds(0, D)]) for t in range(NWC)]
    k0_cp = copy(k_hbm.at[0, 0, pl.ds(k_hbm.shape[2] - W, W), :], k_sc.at[0])
    v0_cp = copy(v_hbm.at[0, 0, pl.ds(v_hbm.shape[2] - W, W), :], v_sc.at[0])
    k_cp = copy(k_hbm.at[0, pl.ds(1, HKV - 1), pl.ds(k_hbm.shape[2] - W, W), :], k_sc.at[pl.ds(1, HKV - 1)])
    v_cp = copy(v_hbm.at[0, pl.ds(1, HKV - 1), pl.ds(v_hbm.shape[2] - W, W), :], v_sc.at[pl.ds(1, HKV - 1)])
    ffn_cps = [copy(wg_hbm, wg_sc), copy(wu_hbm, wu_sc), copy(wd_hbm, wd_sc.at[:, pl.ds(0, D)])]
    out_sem0 = nsem[0]
    nsem[0] += NT + 1

    def out_cp(t):
        r0 = _mult(t * TQ, TQ)
        src_sc, src_off = (row_sc, 2 * TQ) if "pinE" in _DEV else (xo_sc, S)
        return pltpu.make_async_copy(src_sc.at[pl.ds(src_off + r0, TQ), :], out_hbm.at[0, pl.ds(r0, TQ), :],
                                     sems.at[out_sem0 + t])

    order = [c_cp, x_cps[0]] + wma_cps + [wq_cps[0], k0_cp, v0_cp, wq_cps[1], wr_cp,
                                           x_cps[1], wq_cps[2], wo_cps[0], k_cp, v_cp]
    for t in range(1, NWC):
        if t + 2 < NWC:
            order.append(wq_cps[t + 2])
        order.append(wo_cps[t])
    order += wmb_cps + x_cps[2:] + ffn_cps
    for cp in order:
        cp.start()

    _sc = _scope("p0_prologue"); _sc.__enter__()
    c_cp.wait()
    cf = c_sc[...].astype(F32)
    sc16 = jnp.broadcast_to((cf * jax.nn.sigmoid(cf)).astype(BF), (16, D))

    def mod_chunk(c0, n):
        return jnp.dot(sc16, wmod_sc[:, c0:c0 + n], preferred_element_type=F32)[0:8, :]

    x_cps[0].wait()
    x0 = x_sc[0:TQ, :].astype(F32)
    m0 = jnp.mean(x0, axis=-1, keepdims=True)
    xc0 = x0 - m0
    xh0 = xc0 * lax.rsqrt(jnp.mean(xc0 * xc0, axis=-1, keepdims=True) + EPS)

    for t in range(NMA):
        wma_cps[t].wait()
        mod_sc[:, t * MCA:(t + 1) * MCA] = mod_chunk(t * MCA, MCA)
    row_sc[H_OFF:H_OFF + TQ, :] = (xh0 * (1.0 + mod_sc[0:1, D:2 * D]) + mod_sc[0:1, 0:D]).astype(BF)

    def q_proj(hslot, col, qslot):
        h = row_sc[pl.ds(_mult(H_OFF + hslot * TQ, TQ), TQ), :]
        q = jnp.dot(h, wq_sc[:, pl.ds(_mult(col, DH), DH)], preferred_element_type=F32)
        q_sc[qslot] = (q * QSCALE).astype(BF)

    wq_cps[0].wait()
    for m in range(DELTA):
        q_proj(0, m * DH, m % QB)
    _sc.__exit__(None, None, None)

    def a_piece(tile, k, hslot=None):
        r0 = _mult(tile * TQ + k * RP, RP)
        xf = x_sc[pl.ds(r0, RP), :].astype(F32)
        hh = _ln_mod(xf, 1.0 + mod_sc[0:1, D:2 * D], mod_sc[0:1, 0:D])
        hslot = jnp.bitwise_and(tile, 1) if hslot is None else hslot
        row_sc[pl.ds(_mult(H_OFF + hslot * TQ + k * RP, RP), RP), :] = hh.astype(BF)

    def h2_of(xp):
        return _ln_mod(xp.astype(F32), 1.0 + mod_sc[0:1, 4 * D:5 * D], mod_sc[0:1, 3 * D:4 * D])

    out_ref_sc, out_off = (row_sc, 2 * TQ) if "pinE" in _DEV else (xo_sc, S)

    def e_piece(tile, k, best):
        bval, bidx = best
        r0 = _mult(tile * TQ + k * RP, RP)
        att = att_sc[1, pl.ds(_mult(k * RP, RP), RP), :]
        xp = (x_sc[pl.ds(r0, RP), :].astype(F32) + mod_sc[0:1, 2 * D:3 * D] * att).astype(BF)
        xo_sc[pl.ds(r0, RP), :] = xp
        xf = xp.astype(F32)
        xc = xf - jnp.mean(xf, axis=-1, keepdims=True)
        rstd = lax.rsqrt(jnp.mean(xc * xc, axis=-1, keepdims=True) + EPS)
        out = (xf + ep_sc[1:2, :]) + (xc * rstd) * ep_sc[0:1, :]
        out_ref_sc[pl.ds(out_off + r0, RP), :] = out.astype(BF)
        r = jnp.sum(xc * ep_sc[2:3, :], axis=-1, keepdims=True) * rstd + ep_sc[3:4, 0:1]
        rows = r0 + lax.broadcasted_iota(jnp.int32, (RP, 1), 0)
        better = r > bval
        return jnp.where(better, r, bval), jnp.where(better, rows, bidx)

    def slot(j, g, wo_row, b_hslot, b_col, d_mode, side, dk):
        s = lax.dot_general(q_sc[j % QB], k_sc[g], (((1,), (1,)), ((), ())), preferred_element_type=F32)
        if j % dk == 0:
            d = jnp.dot(o_sc[:, 0:dk * DH], wo_sc[pl.ds(_mult(wo_row, DH), dk * DH), 0:D], preferred_element_type=F32)
        if j % dk != 0:
            pass
        elif d_mode == "acc":
            acc_sc[...] += d
        elif d_mode[0] == "finish":
            t = acc_sc[...] + d
            att_sc[d_mode[1]] = t
            acc_sc[...] = t
        elif len(d_mode) == 3:
            acc_sc[...] = jnp.where(d_mode[1], 0.0, acc_sc[...] + d)
        else:
            acc_sc[...] = jnp.where(d_mode[1], 0.0, acc_sc[...]) + d
        for fn in side.get("early", ()):
            fn()
        mx = jnp.max(s, axis=-1, keepdims=True)
        pe = jnp.exp2(s - mx)
        l = jnp.sum(pe, axis=-1, keepdims=True)
        q_proj(b_hslot, b_col, (j + DELTA) % QB)
        o = jnp.dot(pe.astype(BF), v_sc[g], preferred_element_type=F32)
        rl = pl.reciprocal(l, approx=True)
        rl = rl * (2.0 - l * rl)
        o_sc[:, (j % dk) * DH:(j % dk + 1) * DH] = (o * rl).astype(BF)
        for fn in side.get("late", ()):
            fn()

    def tile0_body(t, carry):
        @pl.when(t + 1 < NWC)
        def _():
            pltpu.make_async_copy(wq_hbm.at[:, pl.ds(0, WC)], wq_sc.at[:, pl.ds(0, WC)],
                                  sems.at[wq_sem0 + t + 1]).wait()

        @pl.when(t >= 1)
        def _():
            pltpu.make_async_copy(wo_hbm.at[pl.ds(0, WC), :], wo_sc.at[pl.ds(0, WC), pl.ds(0, D)],
                                  sems.at[wo_sem0 + t - 1]).wait()

        @pl.when(t == 1)
        def _():
            x_cps[1].wait()

        @pl.when(t == 2)
        def _():
            k_cp.wait()
            v_cp.wait()
        tile_a = jnp.minimum(t, 1)
        last = t == NWC - 1
        col = t * WC
        b_col = jnp.where(last, 0, col + WC)
        b_hslot = last.astype(jnp.int32)
        g = lax.shift_right_logical(t, 1)
        for j in range(HPC):
            side = {}
            if j < 3:
                k = jnp.clip(3 * (t - 1) + j, 0, NP - 1)
                side = {"late": [lambda k=k: a_piece(tile_a, k)]}
            wo_row = jnp.maximum(col + (j - DK0) * DH, 0)
            slot(j, g, wo_row, b_hslot, b_col + j * DH, ("restart", t == 0, True), side, DK0)
        return carry

    with _scope("p1_tile0"):
        k0_cp.wait()
        v0_cp.wait()
        lax.fori_loop(0, NWC, tile0_body, 0)
        wo_cps[NWC - 1].wait()
        if DK > DK0:
            o_sc[:, (DK - DK0) * DH:DK * DH] = o_sc[:, 0:DK0 * DH]
            o_sc[:, 0:(DK - DK0) * DH] = jnp.zeros((TQ, (DK - DK0) * DH), BF)

    _sc = _scope("p2_modrest"); _sc.__enter__()
    for cp in wmb_cps:
        cp.wait()
    wr_cp.wait()
    for t in range(4):
        mod_sc[:, 2048 + t * 1024:2048 + (t + 1) * 1024] = mod_chunk(2048 + t * 1024, 1024)
    wrf_sc[...] = jnp.broadcast_to(wr_sc[...].astype(F32).reshape(1, D), (8, D))
    cb1 = 1.0 + mod_sc[0:1, 4 * D:5 * D]
    ep_sc[0:1, :] = mod_sc[0:1, 5 * D:6 * D] * cb1
    ep_sc[1:2, :] = mod_sc[0:1, 5 * D:6 * D] * mod_sc[0:1, 3 * D:4 * D]
    ep_sc[2:3, :] = cb1 * wrf_sc[0:1, :]
    ep_sc[3:4, :] = jnp.broadcast_to(
        jnp.sum(mod_sc[0:1, 3 * D:4 * D] * wrf_sc[0:1, :], axis=-1, keepdims=True), (1, D))
    _sc.__exit__(None, None, None)

    IPT = NS // NSL
    assert IPT == 2 and HPC == DELTA and 2 * HPC == REP
    PPI = NP // IPT
    a_slot = {(k * (NSL - DELTA)) // PPI: k for k in range(PPI)}
    e_slot = {1 + (k * (NSL - 1)) // PPI: k for k in range(PPI)}

    def main_body(it, best):
        tile = lax.shift_right_logical(it, 1)
        part = jnp.bitwise_and(it, 1)
        first = part == 0
        base = part * (NSL * DH)
        nbase = NSL * DH - base
        hs_same = jnp.bitwise_and(tile, 1)
        hs_next = jnp.bitwise_and(tile + part, 1)
        best = list(best)

        @pl.when(first)
        def _():
            @pl.when(tile + 1 < NT)
            def _():
                pltpu.make_async_copy(x_hbm.at[0, pl.ds(0, TQ), :], x_sc.at[pl.ds(0, TQ), :],
                                      sems.at[x_sem0 + tile + 1]).wait()

            @pl.when(tile >= 2)
            def _():
                out_cp(tile - 2).start()
        for j in range(NSL):
            side = {"late": []}
            if j in a_slot and "noA" not in _DEV:
                side["late"].append(lambda k=a_slot[j]: a_piece(jnp.minimum(tile + 1, NT - 1), part * PPI + k))
            if j in e_slot and "noE" not in _DEV:
                def run_e(k=e_slot[j]):
                    best[:] = e_piece(tile - 1, part * PPI + k, best)
                side["late" if "eearly" not in _DEV else "early"] = side.get("late" if "eearly" not in _DEV else "early", []) + [run_e]
            mode = ("finish", 1 - part) if j == 0 else (("restart", first) if j == DK else "acc")
            g = 2 * part + j // REP
            wo_row = base + (j - DK) * DH if j > 0 else (NS - DK) * DH - base
            if j + DELTA < NSL:
                b_hslot, b_col = hs_same, base + (j + DELTA) * DH
            else:
                b_hslot, b_col = hs_next, nbase + (j + DELTA - NSL) * DH
            slot(j, g, wo_row, b_hslot, b_col, mode, side, DK)
        return tuple(best)

    best = (jnp.full((RP, 1), -jnp.inf, F32), jnp.zeros((RP, 1), jnp.int32))
    with _scope("p3_loop"):
        best = lax.fori_loop(IPT, NT * IPT, main_body, best)

    _sc = _scope("p4_lastE"); _sc.__enter__()
    out_cp(NT - 2).start()
    att_sc[1] = acc_sc[...] + jnp.dot(o_sc[...], wo_sc[(NS - DK) * DH:NS * DH, 0:D], preferred_element_type=F32)
    for k in range(NP):
        best = e_piece(NT - 1, k, best)
    out_cp(NT - 1).start()
    _sc.__exit__(None, None, None)

    _sc = _scope("p5_ffn"); _sc.__enter__()
    bval, bidx = best
    gmax = jnp.max(bval, axis=0, keepdims=True)
    idx = jnp.min(jnp.where(bval == gmax, bidx, S))
    r0 = pl.multiple_of((idx // RP) * RP, RP)
    xp = xo_sc[pl.ds(r0, RP), :]
    h2 = h2_of(xp)
    r = jnp.sum(h2 * wrf_sc[0:1, :], axis=-1, keepdims=True)
    for cp in ffn_cps:
        cp.wait()
    h2b = h2.astype(BF)
    gate = jnp.dot(h2b, wg_sc[...], preferred_element_type=F32)
    up = jnp.dot(h2b, wu_sc[...], preferred_element_type=F32)
    act = (gate * jax.nn.sigmoid(gate) * up).astype(BF)
    y = jnp.dot(act, wd_sc[:, 0:D], preferred_element_type=F32) * jax.nn.sigmoid(r)
    rows = r0 + lax.broadcasted_iota(jnp.int32, (RP, 1), 0)
    upd = jnp.where(rows == idx, y, 0.0)
    fixed = (xp.astype(F32) + mod_sc[0:1, 5 * D:6 * D] * (h2 + upd)).astype(BF)
    _sc.__exit__(None, None, None)
    _sc = _scope("p6_out"); _sc.__enter__()
    for t in range(NT):
        out_cp(t).wait()
    row_sc[H_OFF:H_OFF + RP, :] = fixed
    fix_cp = pltpu.make_async_copy(row_sc.at[pl.ds(H_OFF, RP), :], out_hbm.at[0, pl.ds(r0, RP), :],
                                   sems.at[out_sem0 + NT])
    fix_cp.start()
    fix_cp.wait()
    _sc.__exit__(None, None, None)


_NSEM = 2 + NT + 4 + 4 + 8 + 8 + 4 + 3 + NT + 1


@jax.jit
def pallas_adaLN_cond__sliding_block_cached__moe_arch_mod__prompt_kernel(
    A_x: jax.Array,
    A_k_cache: jax.Array,
    A_v_cache: jax.Array,
    A_wq: jax.Array,
    A_wo: jax.Array,
    B_x: jax.Array,
    B_w_r: jax.Array,
    B_w_gate: jax.Array,
    B_w_up: jax.Array,
    B_w_down: jax.Array,
    c: jax.Array,
    w_mod: jax.Array,
):
    del B_x
    any_spec = pl.BlockSpec(memory_space=pl.ANY)
    scratch = [
        pltpu.VMEM((S, D), BF),
        pltpu.VMEM((ROWS, D), BF),
        pltpu.VMEM((D, HQ * DH + PAD), BF),
        pltpu.VMEM((HQ * DH, D + PAD), BF),
        pltpu.VMEM((HKV, W, DH), BF),
        pltpu.VMEM((HKV, W, DH), BF),
        pltpu.VMEM((D, 6 * D + PAD), BF),
        pltpu.VMEM((D, FF), BF),
        pltpu.VMEM((D, FF), BF),
        pltpu.VMEM((FF, D + PAD), BF),
        pltpu.VMEM((1, D), BF),
        pltpu.VMEM((D,), BF),
        pltpu.VMEM((8, 6 * D), F32),
        pltpu.VMEM((8, D), F32),
        pltpu.VMEM((QB, TQ, DH), BF),
        pltpu.VMEM((TQ, DK * DH), BF),
        pltpu.VMEM((TQ, D), F32),
        pltpu.VMEM((2, TQ, D), F32),
        pltpu.VMEM((2 * S, D), BF),
        pltpu.VMEM((8, D), F32),
        pltpu.SemaphoreType.DMA((_NSEM,)),
    ]
    return pl.pallas_call(
        _kernel,
        out_shape=jax.ShapeDtypeStruct(A_x.shape, A_x.dtype),
        in_specs=[any_spec] * 11,
        out_specs=any_spec,
        scratch_shapes=scratch,
        compiler_params=pltpu.CompilerParams(vmem_limit_bytes=100 * 1024 * 1024),
    )(A_x, A_k_cache, A_v_cache, A_wq, A_wo, B_w_r, B_w_gate, B_w_up, B_w_down, c, w_mod)
```

```python
import contextlib

import jax
import jax.numpy as jnp
from jax import lax
import jax.experimental.pallas as pl
import jax.experimental.pallas.tpu as pltpu

BF = jnp.bfloat16
F32 = jnp.float32

S, D = 2048, 1024
HQ, HKV, DH = 32, 4, 128
REP = HQ // HKV
W = 512
FF = 3584
EPS = 1e-5
QSCALE = (DH ** -0.5) * 1.4426950408889634

TQ = 256
NT = S // TQ
NS = HQ
DELTA = 4
QB = 4
NSL = 16
DK0 = 4
DK = 4
PAD = 128
APAD = 0
NPIN = 0
EPAT = 1
ELATE = 1
RE = 16
LASTSPLIT = 4
RP = 16
NP = TQ // RP

H_OFF = 0
ROWS = 2 * TQ

_DEV = set()
_FLAGS = None
_SCOPES = False


def _scope(name):
    return jax.named_scope(name) if _SCOPES else contextlib.nullcontext()


def _ln_mod(xf, scale1, shift):
    m = jnp.mean(xf, axis=-1, keepdims=True)
    xc = xf - m
    v = jnp.mean(xc * xc, axis=-1, keepdims=True)
    return xc * lax.rsqrt(v + EPS) * scale1 + shift


def _mult(v, m):
    return v if isinstance(v, int) else pl.multiple_of(v, m)


def _kernel(x_hbm, k_hbm, v_hbm, wq_hbm, wo_hbm, wr_hbm, wg_hbm, wu_hbm, wd_hbm, c_hbm, wmod_hbm,
            out_hbm,
            x_sc, row_sc, wq_sc, wo_sc, k_sc, v_sc, wmod_sc, wg_sc, wu_sc, wd_sc,
            c_sc, wr_sc, mod_sc, wrf_sc, q_sc, oo_sc, acc_sc, att_sc, xo_sc, ep_sc, sems):

    nsem = [0]

    def copy(src, dst):
        k = nsem[0]
        nsem[0] += 1
        return pltpu.make_async_copy(src, dst, sems.at[k])

    NMA = 4
    MCA = 2048 // NMA
    NMB = 4
    MCB = 4096 // NMB
    NWC = 8
    WC = 4096 // NWC
    HPC = HQ // NWC

    c_cp = copy(c_hbm, c_sc)
    wr_cp = copy(wr_hbm, wr_sc)
    x_sem0 = nsem[0]
    x_cps = [copy(x_hbm.at[0, pl.ds(t * TQ, TQ), :], x_sc.at[pl.ds(t * TQ, TQ), :]) for t in range(NT)]
    wma_cps = [copy(wmod_hbm.at[:, pl.ds(t * MCA, MCA)], wmod_sc.at[:, pl.ds(t * MCA, MCA)]) for t in range(NMA)]
    wmb_cps = [copy(wmod_hbm.at[:, pl.ds(2048 + t * MCB, MCB)], wmod_sc.at[:, pl.ds(2048 + t * MCB, MCB)])
               for t in range(NMB)]
    wq_sem0 = nsem[0]
    wq_cps = [copy(wq_hbm.at[:, pl.ds(t * WC, WC)], wq_sc.at[:, pl.ds(t * WC, WC)]) for t in range(NWC)]
    wo_sem0 = nsem[0]
    wo_cps = [copy(wo_hbm.at[pl.ds(t * WC, WC), :], wo_sc.at[pl.ds(t * WC, WC), pl.ds(0, D)]) for t in range(NWC)]
    k0_cp = copy(k_hbm.at[0, 0, pl.ds(k_hbm.shape[2] - W, W), :], k_sc.at[0])
    v0_cp = copy(v_hbm.at[0, 0, pl.ds(v_hbm.shape[2] - W, W), :], v_sc.at[0])
    k_cp = copy(k_hbm.at[0, pl.ds(1, HKV - 1), pl.ds(k_hbm.shape[2] - W, W), :], k_sc.at[pl.ds(1, HKV - 1)])
    v_cp = copy(v_hbm.at[0, pl.ds(1, HKV - 1), pl.ds(v_hbm.shape[2] - W, W), :], v_sc.at[pl.ds(1, HKV - 1)])
    ffn_cps = [copy(wg_hbm, wg_sc), copy(wu_hbm, wu_sc), copy(wd_hbm, wd_sc.at[:, pl.ds(0, D)])]
    out_sem0 = nsem[0]
    nsem[0] += NT + 1

    def out_cp(t):
        r0 = _mult(t * TQ, TQ)
        src_sc, src_off = (oo_sc, 0) if "pinO" in _DEV else (xo_sc, S)
        return pltpu.make_async_copy(src_sc.at[pl.ds(src_off + r0, TQ), :], out_hbm.at[0, pl.ds(r0, TQ), :],
                                     sems.at[out_sem0 + t])

    order = [c_cp, x_cps[0]] + wma_cps + [wq_cps[0], k0_cp, v0_cp, wq_cps[1], wr_cp,
                                           x_cps[1], wq_cps[2], wo_cps[0], k_cp, v_cp]
    for t in range(1, NWC):
        if t + 2 < NWC:
            order.append(wq_cps[t + 2])
        order.append(wo_cps[t])
    order += wmb_cps + x_cps[2:] + ffn_cps
    for cp in order:
        cp.start()

    _sc = _scope("p0_prologue"); _sc.__enter__()
    c_cp.wait()
    cf = c_sc[...].astype(F32)
    sc16 = jnp.broadcast_to((cf * jax.nn.sigmoid(cf)).astype(BF), (16, D))

    def mod_chunk(c0, n):
        return jnp.dot(sc16, wmod_sc[:, c0:c0 + n], preferred_element_type=F32)[0:8, :]

    x_cps[0].wait()
    x0 = x_sc[0:TQ, :].astype(F32)
    m0 = jnp.mean(x0, axis=-1, keepdims=True)
    xc0 = x0 - m0
    xh0 = xc0 * lax.rsqrt(jnp.mean(xc0 * xc0, axis=-1, keepdims=True) + EPS)

    for t in range(NMA):
        wma_cps[t].wait()
        mod_sc[:, t * MCA:(t + 1) * MCA] = mod_chunk(t * MCA, MCA)
    row_sc[H_OFF:H_OFF + TQ, :] = (xh0 * (1.0 + mod_sc[0:1, D:2 * D]) + mod_sc[0:1, 0:D]).astype(BF)

    def q_proj(hslot, col, qslot):
        h = row_sc[pl.ds(_mult(H_OFF + hslot * TQ, TQ), TQ), :]
        q = jnp.dot(h, wq_sc[:, pl.ds(_mult(col, DH), DH)], preferred_element_type=F32)
        q_sc[qslot] = (q * QSCALE).astype(BF)

    wq_cps[0].wait()
    for m in range(DELTA):
        q_proj(0, m * DH, m % QB)
    _sc.__exit__(None, None, None)

    def a_piece(tile, k, hslot=None):
        r0 = _mult(tile * TQ + k * RP, RP)
        xf = x_sc[pl.ds(r0, RP), :].astype(F32)
        hh = _ln_mod(xf, 1.0 + mod_sc[0:1, D:2 * D], mod_sc[0:1, 0:D])
        hslot = jnp.bitwise_and(tile, 1) if hslot is None else hslot
        row_sc[pl.ds(_mult(H_OFF + hslot * TQ + k * RP, RP), RP), :] = hh.astype(BF)

    def h2_of(xp):
        return _ln_mod(xp.astype(F32), 1.0 + mod_sc[0:1, 4 * D:5 * D], mod_sc[0:1, 3 * D:4 * D])

    out_ref_sc, out_off = (oo_sc, 0) if "pinO" in _DEV else (xo_sc, S)

    def e_piece(tile, k, best, pin=False):
        bval, bidx = best
        r0 = _mult(tile * TQ + k * RE, RE)
        att = att_sc[1, pl.ds(_mult(k * RE, RE), RE), :]
        xp = (x_sc[pl.ds(r0, RE), :].astype(F32) + mod_sc[0:1, 2 * D:3 * D] * att).astype(BF)
        xo_sc[pl.ds(r0, RE), :] = xp
        xf = xp.astype(F32)
        xc = xf - jnp.mean(xf, axis=-1, keepdims=True)
        rstd = lax.rsqrt(jnp.mean(xc * xc, axis=-1, keepdims=True) + EPS)
        out = (xf + ep_sc[1:2, :]) + (xc * rstd) * ep_sc[0:1, :]
        if pin:
            row_sc[pl.ds(2 * TQ + r0, RE), :] = out.astype(BF)
        else:
            out_ref_sc[pl.ds(out_off + r0, RE), :] = out.astype(BF)
        r = jnp.sum(xc * ep_sc[2:3, :], axis=-1, keepdims=True) * rstd + ep_sc[3:4, 0:1]
        rows = r0 + lax.broadcasted_iota(jnp.int32, (RE, 1), 0)
        better = r > bval
        return jnp.where(better, r, bval), jnp.where(better, rows, bidx)

    def slot(j, g, wo_row, b_hslot, b_col, d_mode, side, dk):
        s = lax.dot_general(q_sc[j % QB], k_sc[g], (((1,), (1,)), ((), ())), preferred_element_type=F32)
        if j % dk == 0 and d_mode is not None:
            d = jnp.dot(oo_sc[S:S + TQ, 0:dk * DH], wo_sc[pl.ds(_mult(wo_row, DH), dk * DH), 0:D], preferred_element_type=F32)
        if j % dk != 0 or d_mode is None:
            pass
        elif d_mode == "acc":
            acc_sc[...] += d
        elif d_mode[0] == "finish":
            t = acc_sc[...] + d
            if d_mode[1] is None:
                att_sc[1] = t
            else:
                att_sc[d_mode[1]] = t
                acc_sc[...] = t
        elif d_mode[1] is None:
            acc_sc[...] = d
        else:
            acc_sc[...] = jnp.where(d_mode[1], 0.0, acc_sc[...]) + d
        for fn in side.get("early", ()):
            fn()
        mx = jnp.max(s, axis=-1, keepdims=True)
        pe = jnp.exp2(s - mx)
        l = jnp.sum(pe, axis=-1, keepdims=True)
        q_proj(b_hslot, b_col, (j + DELTA) % QB)
        o = jnp.dot(pe.astype(BF), v_sc[g], preferred_element_type=F32)
        rl = pl.reciprocal(l, approx=True)
        rl = rl * (2.0 - l * rl)
        oo_sc[S:S + TQ, (j % dk) * DH:(j % dk + 1) * DH] = (o * rl).astype(BF)
        for fn in side.get("late", ()):
            fn()

    def tile0_body(t, carry):
        if isinstance(t, int):
            wq_cps[1].wait()
            for j in range(HPC):
                slot(j, 0, 0, 0, WC + j * DH, None, {}, DK0)
            return carry

        @pl.when(t + 1 < NWC)
        def _():
            pltpu.make_async_copy(wq_hbm.at[:, pl.ds(0, WC)], wq_sc.at[:, pl.ds(0, WC)],
                                  sems.at[wq_sem0 + t + 1]).wait()
        pltpu.make_async_copy(wo_hbm.at[pl.ds(0, WC), :], wo_sc.at[pl.ds(0, WC), pl.ds(0, D)],
                              sems.at[wo_sem0 + t - 1]).wait()

        @pl.when(t == 1)
        def _():
            x_cps[1].wait()

        @pl.when(t == 2)
        def _():
            k_cp.wait()
            v_cp.wait()
        last = t == NWC - 1
        col = t * WC
        b_col = jnp.where(last, 0, col + WC)
        b_hslot = last.astype(jnp.int32)
        g = lax.shift_right_logical(t, 1)
        for j in range(HPC):
            side = {}
            if j < 3:
                k = jnp.minimum(3 * (t - 1) + j, NP - 1)
                side = {"late": [lambda k=k: a_piece(1, k)]}
            slot(j, g, col - DK0 * DH, b_hslot, b_col + j * DH, ("restart", t == 1), side, DK0)
        return carry

    with _scope("p1_tile0"):
        k0_cp.wait()
        v0_cp.wait()
        tile0_body(0, 0)
        lax.fori_loop(1, NWC, tile0_body, 0)
        wo_cps[NWC - 1].wait()
        if DK > DK0:
            oo_sc[S:S + TQ, (DK - DK0) * DH:DK * DH] = oo_sc[S:S + TQ, 0:DK0 * DH]
            oo_sc[S:S + TQ, 0:(DK - DK0) * DH] = jnp.zeros((TQ, (DK - DK0) * DH), BF)

    _sc = _scope("p2_modrest"); _sc.__enter__()
    for cp in wmb_cps:
        cp.wait()
    wr_cp.wait()
    for t in range(4):
        mod_sc[:, 2048 + t * 1024:2048 + (t + 1) * 1024] = mod_chunk(2048 + t * 1024, 1024)
    wrf_sc[...] = jnp.broadcast_to(wr_sc[...].astype(F32).reshape(1, D), (8, D))
    cb1 = 1.0 + mod_sc[0:1, 4 * D:5 * D]
    ep_sc[0:1, :] = mod_sc[0:1, 5 * D:6 * D] * cb1
    ep_sc[1:2, :] = mod_sc[0:1, 5 * D:6 * D] * mod_sc[0:1, 3 * D:4 * D]
    ep_sc[2:3, :] = cb1 * wrf_sc[0:1, :]
    ep_sc[3:4, :] = jnp.broadcast_to(
        jnp.sum(mod_sc[0:1, 3 * D:4 * D] * wrf_sc[0:1, :], axis=-1, keepdims=True), (1, D))
    _sc.__exit__(None, None, None)

    IPT = NS // NSL
    assert IPT in (1, 2) and HPC == DELTA and 2 * HPC == REP
    PPI = NP // IPT
    a_slot = {(k * (NSL - DELTA)) // PPI: k for k in range(PPI)}
    PPE = TQ // RE // IPT
    pats = {
        0: [1 + (k * (NSL - 1)) // PPE for k in range(PPE)],
        1: [1 + k // 2 for k in range(PPE)],
        2: [NSL - 1 - (PPE - 1 - k) // 2 for k in range(PPE)],
        3: [2 + (k * (NSL - 6)) // PPE for k in range(PPE)],
        4: [(2, 2, 5, 5, 8, 8, 11, 11)[k % 8] for k in range(PPE)],
        5: [(4, 5, 6, 7, 8, 9, 10, 11)[k % 8] for k in range(PPE)],
        6: [(8, 9, 10, 11, 12, 13, 14, 15)[k % 8] for k in range(PPE)],
    }
    e_slot = {}
    for k, j in enumerate(pats[EPAT]):
        e_slot.setdefault(j, []).append(k)

    def start_of_tile(tile):
        @pl.when(tile + 1 < NT)
        def _():
            pltpu.make_async_copy(x_hbm.at[0, pl.ds(0, TQ), :], x_sc.at[pl.ds(0, TQ), :],
                                  sems.at[x_sem0 + tile + 1]).wait()

        @pl.when(tile >= 2)
        def _():
            out_cp(tile - 2).start()

    def main_body(it, best):
        best = list(best)
        if IPT == 2:
            tile = lax.shift_right_logical(it, 1)
            part = jnp.bitwise_and(it, 1)
            first = part == 0
            base = part * (NSL * DH)
            nbase = NSL * DH - base
            hs_next = jnp.bitwise_and(tile + part, 1)
            pl.when(first)(lambda: start_of_tile(tile))
            finish, restart = ("finish", 1 - part), ("restart", first)
        else:
            tile, part, base, nbase = it, 0, 0, 0
            hs_next = jnp.bitwise_and(tile + 1, 1)
            start_of_tile(tile)
            finish, restart = ("finish", None), ("restart", None)
        hs_same = jnp.bitwise_and(tile, 1)
        for j in range(NSL):
            side = {"late": []}
            if j in a_slot and "noA" not in _DEV:
                side["late"].append(lambda k=a_slot[j]: a_piece(jnp.minimum(tile + 1, NT - 1), part * PPI + k))
            for k in e_slot.get(j, ()) if "noE" not in _DEV else ():
                def run_e(k=k):
                    best[:] = e_piece(tile - 1, part * PPE + k, best, pin=k < NPIN)
                side["late" if ELATE else "early"] = side.get("late" if ELATE else "early", []) + [run_e]
            mode = finish if j == 0 else (restart if j == DK else "acc")
            g = (NSL // REP) * part + j // REP
            wo_row = base + (j - DK) * DH if j > 0 else (NS - DK) * DH - base
            if j + DELTA < NSL:
                b_hslot, b_col = hs_same, base + (j + DELTA) * DH
            else:
                b_hslot, b_col = hs_next, nbase + (j + DELTA - NSL) * DH
            slot(j, g, wo_row, b_hslot, b_col, mode, side, DK)
        return tuple(best)

    best = (jnp.full((RE, 1), -jnp.inf, F32), jnp.zeros((RE, 1), jnp.int32))
    with _scope("p3_loop"):
        best = lax.fori_loop(IPT, NT * IPT, main_body, best)

    _sc = _scope("p4_lastE"); _sc.__enter__()
    out_cp(NT - 2).start()
    HT = TQ // LASTSPLIT
    for hb in range(LASTSPLIT):
        rows = slice(hb * HT, (hb + 1) * HT)
        att_sc[1, rows, :] = acc_sc[rows, :] + jnp.dot(oo_sc[S + hb * HT:S + (hb + 1) * HT, 0:DK * DH],
                                                       wo_sc[(NS - DK) * DH:NS * DH, 0:D],
                                                       preferred_element_type=F32)
    for k in range(TQ // RE):
        best = e_piece(NT - 1, k, best)
    out_cp(NT - 1).start()
    _sc.__exit__(None, None, None)

    _sc = _scope("p5_ffn"); _sc.__enter__()
    bval, bidx = best
    gmax = jnp.max(bval, axis=0, keepdims=True)
    idx = jnp.min(jnp.where(bval == gmax, bidx, S))
    r0 = pl.multiple_of((idx // RP) * RP, RP)
    xp = xo_sc[pl.ds(r0, RP), :]
    h2 = h2_of(xp)
    r = jnp.sum(h2 * wrf_sc[0:1, :], axis=-1, keepdims=True)
    for cp in ffn_cps:
        cp.wait()
    h2b = h2.astype(BF)
    gate = jnp.dot(h2b, wg_sc[...], preferred_element_type=F32)
    up = jnp.dot(h2b, wu_sc[...], preferred_element_type=F32)
    act = (gate * jax.nn.sigmoid(gate) * up).astype(BF)
    y = jnp.dot(act, wd_sc[:, 0:D], preferred_element_type=F32) * jax.nn.sigmoid(r)
    rows = r0 + lax.broadcasted_iota(jnp.int32, (RP, 1), 0)
    upd = jnp.where(rows == idx, y, 0.0)
    fixed = (xp.astype(F32) + mod_sc[0:1, 5 * D:6 * D] * (h2 + upd)).astype(BF)
    _sc.__exit__(None, None, None)
    _sc = _scope("p6_out"); _sc.__enter__()
    for t in range(NT):
        out_cp(t).wait()
    row_sc[H_OFF:H_OFF + RP, :] = fixed
    fix_cp = pltpu.make_async_copy(row_sc.at[pl.ds(H_OFF, RP), :], out_hbm.at[0, pl.ds(r0, RP), :],
                                   sems.at[out_sem0 + NT])
    fix_cp.start()
    fix_cp.wait()
    _sc.__exit__(None, None, None)


_NSEM = 2 + NT + 4 + 4 + 8 + 8 + 4 + 3 + NT + 1


@jax.jit
def pallas_adaLN_cond__sliding_block_cached__moe_arch_mod__prompt_kernel(
    A_x: jax.Array,
    A_k_cache: jax.Array,
    A_v_cache: jax.Array,
    A_wq: jax.Array,
    A_wo: jax.Array,
    B_x: jax.Array,
    B_w_r: jax.Array,
    B_w_gate: jax.Array,
    B_w_up: jax.Array,
    B_w_down: jax.Array,
    c: jax.Array,
    w_mod: jax.Array,
):
    del B_x
    any_spec = pl.BlockSpec(memory_space=pl.ANY)
    scratch = [
        pltpu.VMEM((S, D), BF),
        pltpu.VMEM((ROWS, D), BF),
        pltpu.VMEM((D, HQ * DH + PAD), BF),
        pltpu.VMEM((HQ * DH, D + PAD), BF),
        pltpu.VMEM((HKV, W, DH), BF),
        pltpu.VMEM((HKV, W, DH), BF),
        pltpu.VMEM((D, 6 * D + PAD), BF),
        pltpu.VMEM((D, FF), BF),
        pltpu.VMEM((D, FF), BF),
        pltpu.VMEM((FF, D + PAD), BF),
        pltpu.VMEM((1, D), BF),
        pltpu.VMEM((D,), BF),
        pltpu.VMEM((8, 6 * D), F32),
        pltpu.VMEM((8, D), F32),
        pltpu.VMEM((QB, TQ, DH), BF),
        pltpu.VMEM((S + TQ, D), BF),
        pltpu.VMEM((TQ, D), F32),
        pltpu.VMEM((2, TQ, D), F32),
        pltpu.VMEM((2 * S, D), BF),
        pltpu.VMEM((8, D), F32),
        pltpu.SemaphoreType.DMA((_NSEM,)),
    ]
    return pl.pallas_call(
        _kernel,
        out_shape=jax.ShapeDtypeStruct(A_x.shape, A_x.dtype),
        in_specs=[any_spec] * 11,
        out_specs=any_spec,
        scratch_shapes=scratch,
        compiler_params=pltpu.CompilerParams(vmem_limit_bytes=100 * 1024 * 1024, flags=_FLAGS),
    )(A_x, A_k_cache, A_v_cache, A_wq, A_wo, B_w_r, B_w_gate, B_w_up, B_w_down, c, w_mod)
```

```python
import contextlib

import jax
import jax.numpy as jnp
from jax import lax
import jax.experimental.pallas as pl
import jax.experimental.pallas.tpu as pltpu

BF = jnp.bfloat16
F32 = jnp.float32

S, D = 2048, 1024
HQ, HKV, DH = 32, 4, 128
REP = HQ // HKV
W = 512
FF = 3584
EPS = 1e-5
QSCALE = (DH ** -0.5) * 1.4426950408889634

TQ = 256
NT = S // TQ
NS = HQ
DELTA = 4
QB = 4
NSL = 16
DK0 = 4
DK = 4
PAD = 128
APAD = 0
NPIN = 0
EPAT = 1
ELATE = 1
RE = 16
SORD = 1
DPH = 0
LASTSPLIT = 4
RP = 16
NP = TQ // RP

H_OFF = 0
ROWS = 2 * TQ

_DEV = set()
_FLAGS = None
_SCOPES = False


def _scope(name):
    return jax.named_scope(name) if _SCOPES else contextlib.nullcontext()


def _ln_mod(xf, scale1, shift):
    m = jnp.mean(xf, axis=-1, keepdims=True)
    xc = xf - m
    v = jnp.mean(xc * xc, axis=-1, keepdims=True)
    return xc * lax.rsqrt(v + EPS) * scale1 + shift


def _mult(v, m):
    return v if isinstance(v, int) else pl.multiple_of(v, m)


def _kernel(x_hbm, k_hbm, v_hbm, wq_hbm, wo_hbm, wr_hbm, wg_hbm, wu_hbm, wd_hbm, c_hbm, wmod_hbm,
            out_hbm,
            x_sc, row_sc, wq_sc, wo_sc, k_sc, v_sc, wmod_sc, wg_sc, wu_sc, wd_sc,
            c_sc, wr_sc, mod_sc, wrf_sc, q_sc, oo_sc, acc_sc, att_sc, xo_sc, ep_sc, sems):

    nsem = [0]

    def copy(src, dst):
        k = nsem[0]
        nsem[0] += 1
        return pltpu.make_async_copy(src, dst, sems.at[k])

    NMA = 4
    MCA = 2048 // NMA
    NMB = 4
    MCB = 4096 // NMB
    NWC = 8
    WC = 4096 // NWC
    HPC = HQ // NWC

    c_cp = copy(c_hbm, c_sc)
    wr_cp = copy(wr_hbm, wr_sc)
    x_sem0 = nsem[0]
    x_cps = [copy(x_hbm.at[0, pl.ds(t * TQ, TQ), :], x_sc.at[pl.ds(t * TQ, TQ), :]) for t in range(NT)]
    wma_cps = [copy(wmod_hbm.at[:, pl.ds(t * MCA, MCA)], wmod_sc.at[:, pl.ds(t * MCA, MCA)]) for t in range(NMA)]
    wmb_cps = [copy(wmod_hbm.at[:, pl.ds(2048 + t * MCB, MCB)], wmod_sc.at[:, pl.ds(2048 + t * MCB, MCB)])
               for t in range(NMB)]
    wq_sem0 = nsem[0]
    wq_cps = [copy(wq_hbm.at[:, pl.ds(t * WC, WC)], wq_sc.at[:, pl.ds(t * WC, WC)]) for t in range(NWC)]
    wo_sem0 = nsem[0]
    wo_cps = [copy(wo_hbm.at[pl.ds(t * WC, WC), :], wo_sc.at[pl.ds(t * WC, WC), pl.ds(0, D)]) for t in range(NWC)]
    k0_cp = copy(k_hbm.at[0, 0, pl.ds(k_hbm.shape[2] - W, W), :], k_sc.at[0])
    v0_cp = copy(v_hbm.at[0, 0, pl.ds(v_hbm.shape[2] - W, W), :], v_sc.at[0])
    k_cp = copy(k_hbm.at[0, pl.ds(1, HKV - 1), pl.ds(k_hbm.shape[2] - W, W), :], k_sc.at[pl.ds(1, HKV - 1)])
    v_cp = copy(v_hbm.at[0, pl.ds(1, HKV - 1), pl.ds(v_hbm.shape[2] - W, W), :], v_sc.at[pl.ds(1, HKV - 1)])
    ffn_cps = [copy(wg_hbm, wg_sc), copy(wu_hbm, wu_sc), copy(wd_hbm, wd_sc.at[:, pl.ds(0, D)])]
    out_sem0 = nsem[0]
    nsem[0] += NT + 1

    def out_cp(t):
        r0 = _mult(t * TQ, TQ)
        src_sc, src_off = (oo_sc, 0) if "pinO" in _DEV else (xo_sc, S)
        return pltpu.make_async_copy(src_sc.at[pl.ds(src_off + r0, TQ), :], out_hbm.at[0, pl.ds(r0, TQ), :],
                                     sems.at[out_sem0 + t])

    order = [c_cp, x_cps[0]] + wma_cps + [wq_cps[0], k0_cp, v0_cp, wq_cps[1], wr_cp,
                                           x_cps[1], wq_cps[2], wo_cps[0], k_cp, v_cp]
    for t in range(1, NWC):
        if t + 2 < NWC:
            order.append(wq_cps[t + 2])
        order.append(wo_cps[t])
    order += wmb_cps + x_cps[2:] + ffn_cps
    for cp in order:
        cp.start()

    _sc = _scope("p0_prologue"); _sc.__enter__()
    c_cp.wait()
    cf = c_sc[...].astype(F32)
    sc16 = jnp.broadcast_to((cf * jax.nn.sigmoid(cf)).astype(BF), (16, D))

    def mod_chunk(c0, n):
        return jnp.dot(sc16, wmod_sc[:, c0:c0 + n], preferred_element_type=F32)[0:8, :]

    x_cps[0].wait()
    x0 = x_sc[0:TQ, :].astype(F32)
    m0 = jnp.mean(x0, axis=-1, keepdims=True)
    xc0 = x0 - m0
    xh0 = xc0 * lax.rsqrt(jnp.mean(xc0 * xc0, axis=-1, keepdims=True) + EPS)

    for t in range(NMA):
        wma_cps[t].wait()
        mod_sc[:, t * MCA:(t + 1) * MCA] = mod_chunk(t * MCA, MCA)
    row_sc[H_OFF:H_OFF + TQ, :] = (xh0 * (1.0 + mod_sc[0:1, D:2 * D]) + mod_sc[0:1, 0:D]).astype(BF)

    def q_proj(hslot, col, qslot):
        h = row_sc[pl.ds(_mult(H_OFF + hslot * TQ, TQ), TQ), :]
        q = jnp.dot(h, wq_sc[:, pl.ds(_mult(col, DH), DH)], preferred_element_type=F32)
        q_sc[qslot] = (q * QSCALE).astype(BF)

    wq_cps[0].wait()
    for m in range(DELTA):
        q_proj(0, m * DH, m % QB)
    _sc.__exit__(None, None, None)

    def a_piece(tile, k, hslot=None):
        r0 = _mult(tile * TQ + k * RP, RP)
        xf = x_sc[pl.ds(r0, RP), :].astype(F32)
        hh = _ln_mod(xf, 1.0 + mod_sc[0:1, D:2 * D], mod_sc[0:1, 0:D])
        hslot = jnp.bitwise_and(tile, 1) if hslot is None else hslot
        row_sc[pl.ds(_mult(H_OFF + hslot * TQ + k * RP, RP), RP), :] = hh.astype(BF)

    def h2_of(xp):
        return _ln_mod(xp.astype(F32), 1.0 + mod_sc[0:1, 4 * D:5 * D], mod_sc[0:1, 3 * D:4 * D])

    out_ref_sc, out_off = (oo_sc, 0) if "pinO" in _DEV else (xo_sc, S)

    def e_piece(tile, k, best, pin=False):
        bval, bidx = best
        r0 = _mult(tile * TQ + k * RE, RE)
        att = att_sc[1, pl.ds(_mult(k * RE, RE), RE), :]
        xp = (x_sc[pl.ds(r0, RE), :].astype(F32) + mod_sc[0:1, 2 * D:3 * D] * att).astype(BF)
        xo_sc[pl.ds(r0, RE), :] = xp
        xf = xp.astype(F32)
        xc = xf - jnp.mean(xf, axis=-1, keepdims=True)
        rstd = lax.rsqrt(jnp.mean(xc * xc, axis=-1, keepdims=True) + EPS)
        out = (xf + ep_sc[1:2, :]) + (xc * rstd) * ep_sc[0:1, :]
        if pin:
            row_sc[pl.ds(2 * TQ + r0, RE), :] = out.astype(BF)
        else:
            out_ref_sc[pl.ds(out_off + r0, RE), :] = out.astype(BF)
        r = jnp.sum(xc * ep_sc[2:3, :], axis=-1, keepdims=True) * rstd + ep_sc[3:4, 0:1]
        rows = r0 + lax.broadcasted_iota(jnp.int32, (RE, 1), 0)
        better = r > bval
        return jnp.where(better, r, bval), jnp.where(better, rows, bidx)

    def slot(j, g, wo_row, b_hslot, b_col, d_mode, side, dk, o_rd, o_wr):
        st = {}

        def do_q():
            st["s"] = lax.dot_general(q_sc[j % QB], k_sc[g], (((1,), (1,)), ((), ())), preferred_element_type=F32)

        def do_d():
            if d_mode is not None:
                d = jnp.dot(oo_sc[S:S + TQ, o_rd * DH:(o_rd + dk) * DH], wo_sc[pl.ds(_mult(wo_row, DH), dk * DH), 0:D],
                            preferred_element_type=F32)
                if d_mode == "acc":
                    acc_sc[...] += d
                elif d_mode[0] == "finish":
                    t = acc_sc[...] + d
                    att_sc[d_mode[1]] = t
                    acc_sc[...] = t
                else:
                    acc_sc[...] = jnp.where(d_mode[1], 0.0, acc_sc[...]) + d

        def do_p():
            s = st["s"]
            pe = jnp.exp2(s - jnp.max(s, axis=-1, keepdims=True))
            l = jnp.sum(pe, axis=-1, keepdims=True)
            o = jnp.dot(pe.astype(BF), v_sc[g], preferred_element_type=F32)
            rl = pl.reciprocal(l, approx=True)
            rl = rl * (2.0 - l * rl)
            oo_sc[S:S + TQ, o_wr * DH:(o_wr + 1) * DH] = (o * rl).astype(BF)

        def do_b():
            q_proj(b_hslot, b_col, (j + DELTA) % QB)
        for ch in ("QDBP", "DQBP", "QBDP", "DBQP", "BQDP", "QDPB")[SORD]:
            {"Q": do_q, "D": do_d, "P": do_p, "B": do_b}[ch]()
        for fn in side.get("late", ()):
            fn()

    def tile0_body(t, carry):
        if isinstance(t, int):
            wq_cps[1].wait()
            for j in range(HPC):
                slot(j, 0, 0, 0, WC + j * DH, None, {}, DK0, 4, 4 + j)
            return carry

        @pl.when(t + 1 < NWC)
        def _():
            pltpu.make_async_copy(wq_hbm.at[:, pl.ds(0, WC)], wq_sc.at[:, pl.ds(0, WC)],
                                  sems.at[wq_sem0 + t + 1]).wait()
        pltpu.make_async_copy(wo_hbm.at[pl.ds(0, WC), :], wo_sc.at[pl.ds(0, WC), pl.ds(0, D)],
                              sems.at[wo_sem0 + t - 1]).wait()

        @pl.when(t == 1)
        def _():
            x_cps[1].wait()

        @pl.when(t == 2)
        def _():
            k_cp.wait()
            v_cp.wait()
        last = t == NWC - 1
        col = t * WC
        b_col = jnp.where(last, 0, col + WC)
        b_hslot = last.astype(jnp.int32)
        g = lax.shift_right_logical(t, 1)
        for j in range(HPC):
            side = {}
            if j < 3:
                k = jnp.minimum(3 * (t - 1) + j, NP - 1)
                side = {"late": [lambda k=k: a_piece(1, k)]}
            slot(j, g, col - DK0 * DH, b_hslot, b_col + j * DH, ("restart", t == 1) if j == 0 else None, side,
                 DK0, 4, 4 + j)
        return carry

    with _scope("p1_tile0"):
        k0_cp.wait()
        v0_cp.wait()
        tile0_body(0, 0)
        lax.fori_loop(1, NWC, tile0_body, 0)
        wo_cps[NWC - 1].wait()

    _sc = _scope("p2_modrest"); _sc.__enter__()
    for cp in wmb_cps:
        cp.wait()
    wr_cp.wait()
    for t in range(4):
        mod_sc[:, 2048 + t * 1024:2048 + (t + 1) * 1024] = mod_chunk(2048 + t * 1024, 1024)
    wrf_sc[...] = jnp.broadcast_to(wr_sc[...].astype(F32).reshape(1, D), (8, D))
    cb1 = 1.0 + mod_sc[0:1, 4 * D:5 * D]
    ep_sc[0:1, :] = mod_sc[0:1, 5 * D:6 * D] * cb1
    ep_sc[1:2, :] = mod_sc[0:1, 5 * D:6 * D] * mod_sc[0:1, 3 * D:4 * D]
    ep_sc[2:3, :] = cb1 * wrf_sc[0:1, :]
    ep_sc[3:4, :] = jnp.broadcast_to(
        jnp.sum(mod_sc[0:1, 3 * D:4 * D] * wrf_sc[0:1, :], axis=-1, keepdims=True), (1, D))
    _sc.__exit__(None, None, None)

    IPT = NS // NSL
    assert DK == 4 and DK0 == 4 and IPT in (1, 2) and HPC == DELTA and 2 * HPC == REP
    PPI = NP // IPT
    a_slot = {(k * (NSL - DELTA)) // PPI: k for k in range(PPI)}
    PPE = TQ // RE // IPT
    pats = {
        0: [1 + (k * (NSL - 1)) // PPE for k in range(PPE)],
        1: [1 + k // 2 for k in range(PPE)],
        2: [NSL - 1 - (PPE - 1 - k) // 2 for k in range(PPE)],
        3: [2 + (k * (NSL - 6)) // PPE for k in range(PPE)],
        4: [(2, 2, 5, 5, 8, 8, 11, 11)[k % 8] for k in range(PPE)],
        5: [(4, 5, 6, 7, 8, 9, 10, 11)[k % 8] for k in range(PPE)],
        6: [(8, 9, 10, 11, 12, 13, 14, 15)[k % 8] for k in range(PPE)],
    }
    e_slot = {}
    for k, j in enumerate(pats[EPAT]):
        e_slot.setdefault(j, []).append(k)

    def start_of_tile(tile):
        @pl.when(tile + 1 < NT)
        def _():
            pltpu.make_async_copy(x_hbm.at[0, pl.ds(0, TQ), :], x_sc.at[pl.ds(0, TQ), :],
                                  sems.at[x_sem0 + tile + 1]).wait()

        @pl.when(tile >= 2)
        def _():
            out_cp(tile - 2).start()

    def main_body(it, best):
        best = list(best)
        if IPT == 2:
            tile = lax.shift_right_logical(it, 1)
            part = jnp.bitwise_and(it, 1)
            first = part == 0
            base = part * (NSL * DH)
            nbase = NSL * DH - base
            hs_next = jnp.bitwise_and(tile + part, 1)
            pl.when(first)(lambda: start_of_tile(tile))
            finish, restart = ("finish", 1 - part), ("restart", first)
        else:
            tile, part, base, nbase = it, 0, 0, 0
            hs_next = jnp.bitwise_and(tile + 1, 1)
            start_of_tile(tile)
            finish, restart = ("finish", None), ("restart", None)
        hs_same = jnp.bitwise_and(tile, 1)
        for j in range(NSL):
            side = {"late": []}
            if j in a_slot and "noA" not in _DEV:
                side["late"].append(lambda k=a_slot[j]: a_piece(jnp.minimum(tile + 1, NT - 1), part * PPI + k))
            for k in e_slot.get(j, ()) if "noE" not in _DEV else ():
                def run_e(k=k):
                    best[:] = e_piece(tile - 1, part * PPE + k, best, pin=k < NPIN)
                side["late" if ELATE else "early"] = side.get("late" if ELATE else "early", []) + [run_e]
            mode = None if j % DK != DPH else (finish if j == DPH else (restart if j == DPH + DK else "acc"))
            g = (NSL // REP) * part + j // REP
            wo_row = base + (j - DPH - DK) * DH if j > DPH else (NS - DK) * DH - base
            if j + DELTA < NSL:
                b_hslot, b_col = hs_same, base + (j + DELTA) * DH
            else:
                b_hslot, b_col = hs_next, nbase + (j + DELTA - NSL) * DH
            slot(j, g, wo_row, b_hslot, b_col, mode, side, DK, (j - DPH - DK) % 8, j % 8)
        return tuple(best)

    best = (jnp.full((RE, 1), -jnp.inf, F32), jnp.zeros((RE, 1), jnp.int32))
    with _scope("p3_loop"):
        best = lax.fori_loop(IPT, NT * IPT, main_body, best)

    _sc = _scope("p4_lastE"); _sc.__enter__()
    out_cp(NT - 2).start()
    HT = TQ // LASTSPLIT
    for hb in range(LASTSPLIT):
        rows = slice(hb * HT, (hb + 1) * HT)
        att_sc[1, rows, :] = acc_sc[rows, :] + jnp.dot(oo_sc[S + hb * HT:S + (hb + 1) * HT, 4 * DH:8 * DH],
                                                       wo_sc[(NS - DK) * DH:NS * DH, 0:D],
                                                       preferred_element_type=F32)
    for k in range(TQ // RE):
        best = e_piece(NT - 1, k, best)
    out_cp(NT - 1).start()
    _sc.__exit__(None, None, None)

    _sc = _scope("p5_ffn"); _sc.__enter__()
    bval, bidx = best
    gmax = jnp.max(bval, axis=0, keepdims=True)
    idx = jnp.min(jnp.where(bval == gmax, bidx, S))
    r0 = pl.multiple_of((idx // RP) * RP, RP)
    xp = xo_sc[pl.ds(r0, RP), :]
    h2 = h2_of(xp)
    r = jnp.sum(h2 * wrf_sc[0:1, :], axis=-1, keepdims=True)
    for cp in ffn_cps:
        cp.wait()
    h2b = h2.astype(BF)
    gate = jnp.dot(h2b, wg_sc[...], preferred_element_type=F32)
    up = jnp.dot(h2b, wu_sc[...], preferred_element_type=F32)
    act = (gate * jax.nn.sigmoid(gate) * up).astype(BF)
    y = jnp.dot(act, wd_sc[:, 0:D], preferred_element_type=F32) * jax.nn.sigmoid(r)
    rows = r0 + lax.broadcasted_iota(jnp.int32, (RP, 1), 0)
    upd = jnp.where(rows == idx, y, 0.0)
    fixed = (xp.astype(F32) + mod_sc[0:1, 5 * D:6 * D] * (h2 + upd)).astype(BF)
    _sc.__exit__(None, None, None)
    _sc = _scope("p6_out"); _sc.__enter__()
    for t in range(NT):
        out_cp(t).wait()
    row_sc[H_OFF:H_OFF + RP, :] = fixed
    fix_cp = pltpu.make_async_copy(row_sc.at[pl.ds(H_OFF, RP), :], out_hbm.at[0, pl.ds(r0, RP), :],
                                   sems.at[out_sem0 + NT])
    fix_cp.start()
    fix_cp.wait()
    _sc.__exit__(None, None, None)


_NSEM = 2 + NT + 4 + 4 + 8 + 8 + 4 + 3 + NT + 1


@jax.jit
def pallas_adaLN_cond__sliding_block_cached__moe_arch_mod__prompt_kernel(
    A_x: jax.Array,
    A_k_cache: jax.Array,
    A_v_cache: jax.Array,
    A_wq: jax.Array,
    A_wo: jax.Array,
    B_x: jax.Array,
    B_w_r: jax.Array,
    B_w_gate: jax.Array,
    B_w_up: jax.Array,
    B_w_down: jax.Array,
    c: jax.Array,
    w_mod: jax.Array,
):
    del B_x
    any_spec = pl.BlockSpec(memory_space=pl.ANY)
    scratch = [
        pltpu.VMEM((S, D), BF),
        pltpu.VMEM((ROWS, D), BF),
        pltpu.VMEM((D, HQ * DH + PAD), BF),
        pltpu.VMEM((HQ * DH, D + PAD), BF),
        pltpu.VMEM((HKV, W, DH), BF),
        pltpu.VMEM((HKV, W, DH), BF),
        pltpu.VMEM((D, 6 * D + PAD), BF),
        pltpu.VMEM((D, FF), BF),
        pltpu.VMEM((D, FF), BF),
        pltpu.VMEM((FF, D + PAD), BF),
        pltpu.VMEM((1, D), BF),
        pltpu.VMEM((D,), BF),
        pltpu.VMEM((8, 6 * D), F32),
        pltpu.VMEM((8, D), F32),
        pltpu.VMEM((QB, TQ, DH), BF),
        pltpu.VMEM((S + TQ, D), BF),
        pltpu.VMEM((TQ, D), F32),
        pltpu.VMEM((2, TQ, D), F32),
        pltpu.VMEM((2 * S, D), BF),
        pltpu.VMEM((8, D), F32),
        pltpu.SemaphoreType.DMA((_NSEM,)),
    ]
    return pl.pallas_call(
        _kernel,
        out_shape=jax.ShapeDtypeStruct(A_x.shape, A_x.dtype),
        in_specs=[any_spec] * 11,
        out_specs=any_spec,
        scratch_shapes=scratch,
        compiler_params=pltpu.CompilerParams(vmem_limit_bytes=100 * 1024 * 1024, flags=_FLAGS),
    )(A_x, A_k_cache, A_v_cache, A_wq, A_wo, B_w_r, B_w_gate, B_w_up, B_w_down, c, w_mod)
```

```python
import jax
import jax.numpy as jnp
from jax import lax
import jax.experimental.pallas as pl
import jax.experimental.pallas.tpu as pltpu

BF = jnp.bfloat16
F32 = jnp.float32

S, D = 2048, 1024
HQ, HKV, DH = 32, 4, 128
REP = HQ // HKV
W = 512
FF = 3584
EPS = 1e-5
QSCALE = (DH ** -0.5) * 1.4426950408889634

TQ = 256
NT = S // TQ
DK = 4
NSL = 16
NWC = HQ // DK
WC = DK * DH
RP = 16
NP = TQ // RP
PPI = NP // 2
PAD = 128
NMA, NMB = 4, 4
LASTSPLIT = 4
NSEM = 2 + NT + NMA + NMB + 2 * NWC + 4 + 3 + NT + 1


def _dot(a, b):
    return jnp.dot(a, b, preferred_element_type=F32)


def _normalize(xf):
    xc = xf - jnp.mean(xf, axis=-1, keepdims=True)
    return xc, lax.rsqrt(jnp.mean(xc * xc, axis=-1, keepdims=True) + EPS)


def _mult(v, m):
    return v if isinstance(v, int) else pl.multiple_of(v, m)


def _kernel(x_hbm, k_hbm, v_hbm, wq_hbm, wo_hbm, wr_hbm, wg_hbm, wu_hbm, wd_hbm, c_hbm, wmod_hbm,
            out_hbm,
            h_sc, q_sc, o_sc, acc_sc, att_sc, k_sc, v_sc, wq_sc, wo_sc, x_sc, xo_sc,
            wmod_sc, wg_sc, wu_sc, wd_sc, mod_sc, ep_sc, c_sc, wr_sc, sems):

    nsem = [0]

    def copy(src, dst):
        nsem[0] += 1
        return pltpu.make_async_copy(src, dst, sems.at[nsem[0] - 1])

    def wait_like(src, dst, sem_index):
        pltpu.make_async_copy(src, dst, sems.at[sem_index]).wait()

    def cols(ref, c0, n):
        return ref.at[:, pl.ds(c0, n)]

    kv0 = k_hbm.shape[2] - W
    MCA, MCB = 2048 // NMA, 4096 // NMB
    c_cp = copy(c_hbm, c_sc)
    wr_cp = copy(wr_hbm, wr_sc)
    x_sem = nsem[0]
    x_cps = [copy(x_hbm.at[0, pl.ds(t * TQ, TQ), :], x_sc.at[pl.ds(t * TQ, TQ), :]) for t in range(NT)]
    wma_cps = [copy(cols(wmod_hbm, t * MCA, MCA), cols(wmod_sc, t * MCA, MCA)) for t in range(NMA)]
    wmb_cps = [copy(cols(wmod_hbm, 2048 + t * MCB, MCB), cols(wmod_sc, 2048 + t * MCB, MCB)) for t in range(NMB)]
    wq_sem = nsem[0]
    wq_cps = [copy(cols(wq_hbm, t * WC, WC), cols(wq_sc, t * WC, WC)) for t in range(NWC)]
    wo_sem = nsem[0]
    wo_cps = [copy(wo_hbm.at[pl.ds(t * WC, WC), :], wo_sc.at[pl.ds(t * WC, WC), pl.ds(0, D)]) for t in range(NWC)]
    k0_cp = copy(k_hbm.at[0, 0, pl.ds(kv0, W), :], k_sc.at[0])
    v0_cp = copy(v_hbm.at[0, 0, pl.ds(kv0, W), :], v_sc.at[0])
    k_cp = copy(k_hbm.at[0, pl.ds(1, HKV - 1), pl.ds(kv0, W), :], k_sc.at[pl.ds(1, HKV - 1)])
    v_cp = copy(v_hbm.at[0, pl.ds(1, HKV - 1), pl.ds(kv0, W), :], v_sc.at[pl.ds(1, HKV - 1)])
    ffn_cps = [copy(wg_hbm, wg_sc), copy(wu_hbm, wu_sc), copy(wd_hbm, wd_sc.at[:, pl.ds(0, D)])]
    out_sem = nsem[0]

    def out_cp(t):
        r0 = _mult(t * TQ, TQ)
        return pltpu.make_async_copy(xo_sc.at[pl.ds(S + r0, TQ), :], out_hbm.at[0, pl.ds(r0, TQ), :],
                                     sems.at[out_sem + t])

    order = [c_cp, x_cps[0]] + wma_cps + [wq_cps[0], k0_cp, v0_cp, wq_cps[1], wr_cp,
                                           x_cps[1], wq_cps[2], wo_cps[0], k_cp, v_cp]
    for t in range(1, NWC):
        order += [wq_cps[t + 2]] if t + 2 < NWC else []
        order += [wo_cps[t]]
    for cp in order + wmb_cps + x_cps[2:] + ffn_cps:
        cp.start()

    c_cp.wait()
    cf = c_sc[...].astype(F32)
    c16 = jnp.broadcast_to((cf * jax.nn.sigmoid(cf)).astype(BF), (16, D))

    def mod_cols(c0, n):
        mod_sc[:, c0:c0 + n] = _dot(c16, wmod_sc[:, c0:c0 + n])[0:8, :]

    def mod(i):
        return mod_sc[0:1, i * D:(i + 1) * D]

    x_cps[0].wait()
    xc0, rstd0 = _normalize(x_sc[0:TQ, :].astype(F32))
    xh0 = xc0 * rstd0
    for t in range(NMA):
        wma_cps[t].wait()
        mod_cols(t * MCA, MCA)
    h_sc[0:TQ, :] = (xh0 * (1.0 + mod(1)) + mod(0)).astype(BF)

    def q_proj(hslot, col, qslot):
        h = h_sc[pl.ds(_mult(hslot * TQ, TQ), TQ), :]
        q_sc[qslot] = (_dot(h, wq_sc[:, pl.ds(_mult(col, DH), DH)]) * QSCALE).astype(BF)

    wq_cps[0].wait()
    for m in range(DK):
        q_proj(0, m * DH, m)

    def ln1_piece(tile, k):
        xc, rstd = _normalize(x_sc[pl.ds(_mult(tile * TQ + k * RP, RP), RP), :].astype(F32))
        hslot = tile % 2 if isinstance(tile, int) else jnp.bitwise_and(tile, 1)
        h_sc[pl.ds(_mult(hslot * TQ + k * RP, RP), RP), :] = (xc * rstd * (1.0 + mod(1)) + mod(0)).astype(BF)

    def epilogue_piece(tile, k, best):
        bval, bidx = best
        r0 = _mult(tile * TQ + k * RP, RP)
        att = att_sc[1, pl.ds(_mult(k * RP, RP), RP), :]
        xp = (x_sc[pl.ds(r0, RP), :].astype(F32) + mod(2) * att).astype(BF)
        xo_sc[pl.ds(r0, RP), :] = xp
        xf = xp.astype(F32)
        xc, rstd = _normalize(xf)
        xo_sc[pl.ds(S + r0, RP), :] = ((xf + ep_sc[1:2, :]) + (xc * rstd) * ep_sc[0:1, :]).astype(BF)
        r = jnp.sum(xc * ep_sc[2:3, :], axis=-1, keepdims=True) * rstd + ep_sc[3:4, 0:1]
        rows = r0 + lax.broadcasted_iota(jnp.int32, (RP, 1), 0)
        better = r > bval
        return jnp.where(better, r, bval), jnp.where(better, rows, bidx)

    def slot(j, g, b_hslot, b_col, o_wr, proj=None):
        if proj is not None:
            o_rd, wo_row, update = proj
            update(_dot(o_sc[:, o_rd * DH:(o_rd + DK) * DH], wo_sc[pl.ds(_mult(wo_row, DH), WC), 0:D]))
        s = lax.dot_general(q_sc[j % DK], k_sc[g], (((1,), (1,)), ((), ())), preferred_element_type=F32)
        q_proj(b_hslot, b_col, j % DK)
        p = jnp.exp2(s - jnp.max(s, axis=-1, keepdims=True))
        l = jnp.sum(p, axis=-1, keepdims=True)
        o = _dot(p.astype(BF), v_sc[g])
        rl = pl.reciprocal(l, approx=True)
        rl = rl * (2.0 - l * rl)
        o_sc[:, o_wr * DH:(o_wr + 1) * DH] = (o * rl).astype(BF)

    def accumulate(d):
        acc_sc[...] += d

    def restart_unless(keep):
        def update(d):
            acc_sc[...] = jnp.where(keep, acc_sc[...], 0.0) + d
        return update

    k0_cp.wait()
    v0_cp.wait()
    wq_cps[1].wait()
    for j in range(DK):
        slot(j, 0, 0, WC + j * DH, 4 + j)

    def tile0_chunk(t, carry):
        @pl.when(t + 1 < NWC)
        def _():
            wait_like(cols(wq_hbm, 0, WC), cols(wq_sc, 0, WC), wq_sem + t + 1)
        wait_like(wo_hbm.at[pl.ds(0, WC), :], wo_sc.at[pl.ds(0, WC), pl.ds(0, D)], wo_sem + t - 1)

        @pl.when(t == 1)
        def _():
            x_cps[1].wait()

        @pl.when(t == 2)
        def _():
            k_cp.wait()
            v_cp.wait()
        last = t == NWC - 1
        col = t * WC
        b_col = jnp.where(last, 0, col + WC)
        b_hslot = last.astype(jnp.int32)
        g = lax.shift_right_logical(t, 1)
        for j in range(DK):
            proj = (4, col - WC, restart_unless(t > 1)) if j == 0 else None
            slot(j, g, b_hslot, b_col + j * DH, 4 + j, proj)
            if j < 3:
                ln1_piece(1, jnp.minimum(3 * (t - 1) + j, NP - 1))
        return carry

    lax.fori_loop(1, NWC, tile0_chunk, 0)
    wo_cps[NWC - 1].wait()

    for cp in wmb_cps:
        cp.wait()
    wr_cp.wait()
    for t in range(4):
        mod_cols(2048 + t * 1024, 1024)
    wr = wr_sc[...].astype(F32).reshape(1, D)
    cb1 = 1.0 + mod(4)
    ep_sc[0:1, :] = mod(5) * cb1
    ep_sc[1:2, :] = mod(5) * mod(3)
    ep_sc[2:3, :] = cb1 * wr
    ep_sc[3:4, :] = jnp.broadcast_to(jnp.sum(mod(3) * wr, axis=-1, keepdims=True), (1, D))

    ln1_slot = {(k * (NSL - DK)) // PPI: k for k in range(PPI)}
    epi_slot = {1 + k: (2 * k, 2 * k + 1) for k in range(PPI // 2)}

    def main_body(it, best):
        tile = lax.shift_right_logical(it, 1)
        part = jnp.bitwise_and(it, 1)
        first = part == 0

        @pl.when(first)
        def _():
            @pl.when(tile + 1 < NT)
            def _():
                wait_like(x_hbm.at[0, pl.ds(0, TQ), :], x_sc.at[pl.ds(0, TQ), :], x_sem + tile + 1)

            @pl.when(tile >= 2)
            def _():
                out_cp(tile - 2).start()

        base = part * (NSL * DH)
        nbase = NSL * DH - base
        hs_same = jnp.bitwise_and(tile, 1)
        hs_next = jnp.bitwise_and(tile + part, 1)

        def finish(d):
            t = acc_sc[...] + d
            att_sc[1 - part] = t
            acc_sc[...] = t

        for j in range(NSL):
            if j == 0:
                proj = (4, (HQ - DK) * DH - base, finish)
            elif j % DK == 0:
                update = restart_unless(jnp.logical_not(first)) if j == DK else accumulate
                proj = ((j - DK) % 8, base + (j - DK) * DH, update)
            else:
                proj = None
            if j + DK < NSL:
                b_hslot, b_col = hs_same, base + (j + DK) * DH
            else:
                b_hslot, b_col = hs_next, nbase + (j + DK - NSL) * DH
            slot(j, (NSL // REP) * part + j // REP, b_hslot, b_col, j % 8, proj)
            if j in ln1_slot:
                ln1_piece(jnp.minimum(tile + 1, NT - 1), part * PPI + ln1_slot[j])
            for k in epi_slot.get(j, ()):
                best = epilogue_piece(tile - 1, part * PPI + k, best)
        return best

    best = (jnp.full((RP, 1), -jnp.inf, F32), jnp.zeros((RP, 1), jnp.int32))
    best = lax.fori_loop(2, 2 * NT, main_body, best)

    out_cp(NT - 2).start()
    HT = TQ // LASTSPLIT
    for b in range(LASTSPLIT):
        rows = slice(b * HT, (b + 1) * HT)
        att_sc[1, rows, :] = acc_sc[rows, :] + _dot(o_sc[rows, 4 * DH:8 * DH], wo_sc[(HQ - DK) * DH:HQ * DH, 0:D])
    for k in range(NP):
        best = epilogue_piece(NT - 1, k, best)
    out_cp(NT - 1).start()

    bval, bidx = best
    idx = jnp.min(jnp.where(bval == jnp.max(bval, axis=0, keepdims=True), bidx, S))
    r0 = pl.multiple_of((idx // RP) * RP, RP)
    xf = xo_sc[pl.ds(r0, RP), :].astype(F32)
    xc, rstd = _normalize(xf)
    h2 = xc * rstd * cb1 + mod(3)
    r = jnp.sum(h2 * wr, axis=-1, keepdims=True)
    for cp in ffn_cps:
        cp.wait()
    h2b = h2.astype(BF)
    gate = _dot(h2b, wg_sc[...])
    up = _dot(h2b, wu_sc[...])
    act = (gate * jax.nn.sigmoid(gate) * up).astype(BF)
    y = _dot(act, wd_sc[:, 0:D]) * jax.nn.sigmoid(r)
    rows = r0 + lax.broadcasted_iota(jnp.int32, (RP, 1), 0)
    h_sc[0:RP, :] = (xf + mod(5) * (h2 + jnp.where(rows == idx, y, 0.0))).astype(BF)
    for t in range(NT):
        out_cp(t).wait()
    fix_cp = pltpu.make_async_copy(h_sc.at[pl.ds(0, RP), :], out_hbm.at[0, pl.ds(r0, RP), :], sems.at[out_sem + NT])
    fix_cp.start()
    fix_cp.wait()


@jax.jit
def pallas_adaLN_cond__sliding_block_cached__moe_arch_mod__prompt_kernel(
    A_x: jax.Array,
    A_k_cache: jax.Array,
    A_v_cache: jax.Array,
    A_wq: jax.Array,
    A_wo: jax.Array,
    B_x: jax.Array,
    B_w_r: jax.Array,
    B_w_gate: jax.Array,
    B_w_up: jax.Array,
    B_w_down: jax.Array,
    c: jax.Array,
    w_mod: jax.Array,
):
    del B_x
    any_spec = pl.BlockSpec(memory_space=pl.ANY)
    scratch = [
        pltpu.VMEM((2 * TQ, D), BF),
        pltpu.VMEM((DK, TQ, DH), BF),
        pltpu.VMEM((TQ, 2 * WC), BF),
        pltpu.VMEM((TQ, D), F32),
        pltpu.VMEM((2, TQ, D), F32),
        pltpu.VMEM((HKV, W, DH), BF),
        pltpu.VMEM((HKV, W, DH), BF),
        pltpu.VMEM((D, HQ * DH + PAD), BF),
        pltpu.VMEM((HQ * DH, D + PAD), BF),
        pltpu.VMEM((S, D), BF),
        pltpu.VMEM((2 * S, D), BF),
        pltpu.VMEM((D, 6 * D + PAD), BF),
        pltpu.VMEM((D, FF), BF),
        pltpu.VMEM((D, FF), BF),
        pltpu.VMEM((FF, D + PAD), BF),
        pltpu.VMEM((8, 6 * D), F32),
        pltpu.VMEM((8, D), F32),
        pltpu.VMEM((1, D), BF),
        pltpu.VMEM((D,), BF),
        pltpu.SemaphoreType.DMA((NSEM,)),
    ]
    return pl.pallas_call(
        _kernel,
        out_shape=jax.ShapeDtypeStruct(A_x.shape, A_x.dtype),
        in_specs=[any_spec] * 11,
        out_specs=any_spec,
        scratch_shapes=scratch,
        compiler_params=pltpu.CompilerParams(vmem_limit_bytes=100 * 1024 * 1024),
    )(A_x, A_k_cache, A_v_cache, A_wq, A_wo, B_w_r, B_w_gate, B_w_up, B_w_down, c, w_mod)
```

```python
import jax
import jax.numpy as jnp
from jax import lax
import jax.experimental.pallas as pl
import jax.experimental.pallas.tpu as pltpu

BF = jnp.bfloat16
F32 = jnp.float32

S, D = 2048, 1024
HQ, HKV, DH = 32, 4, 128
REP = HQ // HKV
W = 512
FF = 3584
EPS = 1e-5
QSCALE = (DH ** -0.5) * 1.4426950408889634

TQ = 256
NT = S // TQ
DK = 4
NSL = 16
NWC = HQ // DK
WC = DK * DH
RP = 16
NP = TQ // RP
PPI = NP // 2
PAD = 128
NMA, NMB = 4, 4
LASTSPLIT = 4
NSEM = 2 + NT + NMA + NMB + 2 * NWC + 4 + 3 + NT + 1


def _dot(a, b):
    return jnp.dot(a, b, preferred_element_type=F32)


def _pk(v):
    return pltpu.bitcast(v, jnp.uint32)


def _ld(ref_value):
    return pltpu.bitcast(ref_value, BF)


def _half(v):
    return v // 2 if isinstance(v, int) else lax.shift_right_logical(v, 1)


def _normalize(xf):
    xc = xf - jnp.mean(xf, axis=-1, keepdims=True)
    return xc, lax.rsqrt(jnp.mean(xc * xc, axis=-1, keepdims=True) + EPS)


def _mult(v, m):
    return v if isinstance(v, int) else pl.multiple_of(v, m)


def _kernel(x_hbm, k_hbm, v_hbm, wq_hbm, wo_hbm, wr_hbm, wg_hbm, wu_hbm, wd_hbm, c_hbm, wmod_hbm,
            out_hbm,
            h_sc, q_sc, o_sc, acc_sc, att_sc, k_sc, v_sc, wq_sc, wo_sc, x_sc, xo_sc,
            wmod_sc, wg_sc, wu_sc, wd_sc, mod_sc, ep_sc, c_sc, wr_sc, sems):

    nsem = [0]

    def copy(src, dst):
        nsem[0] += 1
        return pltpu.make_async_copy(src, dst, sems.at[nsem[0] - 1])

    def wait_like(src, dst, sem_index):
        pltpu.make_async_copy(src, dst, sems.at[sem_index]).wait()

    def cols(ref, c0, n):
        return ref.at[:, pl.ds(c0, n)]

    kv0 = k_hbm.shape[2] - W
    MCA, MCB = 2048 // NMA, 4096 // NMB
    c_cp = copy(c_hbm, c_sc)
    wr_cp = copy(wr_hbm, wr_sc)
    x_sem = nsem[0]
    x_cps = [copy(x_hbm.at[0, pl.ds(t * TQ, TQ), :], x_sc.at[pl.ds(t * TQ, TQ), :]) for t in range(NT)]
    wma_cps = [copy(cols(wmod_hbm, t * MCA, MCA), cols(wmod_sc, t * MCA, MCA)) for t in range(NMA)]
    wmb_cps = [copy(cols(wmod_hbm, 2048 + t * MCB, MCB), cols(wmod_sc, 2048 + t * MCB, MCB)) for t in range(NMB)]
    wq_sem = nsem[0]
    wq_cps = [copy(cols(wq_hbm, t * WC, WC), cols(wq_sc.bitcast(BF), t * WC, WC)) for t in range(NWC)]
    wo_sem = nsem[0]
    wo_cps = [copy(wo_hbm.at[pl.ds(t * WC, WC), :], wo_sc.bitcast(BF).at[pl.ds(t * WC, WC), pl.ds(0, D)]) for t in range(NWC)]
    k0_cp = copy(k_hbm.at[0, 0, pl.ds(kv0, W), :], k_sc.at[0])
    v0_cp = copy(v_hbm.at[0, 0, pl.ds(kv0, W), :], v_sc.at[0])
    k_cp = copy(k_hbm.at[0, pl.ds(1, HKV - 1), pl.ds(kv0, W), :], k_sc.at[pl.ds(1, HKV - 1)])
    v_cp = copy(v_hbm.at[0, pl.ds(1, HKV - 1), pl.ds(kv0, W), :], v_sc.at[pl.ds(1, HKV - 1)])
    ffn_cps = [copy(wg_hbm, wg_sc), copy(wu_hbm, wu_sc), copy(wd_hbm, wd_sc.at[:, pl.ds(0, D)])]
    out_sem = nsem[0]

    def out_cp(t):
        r0 = _mult(t * TQ, TQ)
        return pltpu.make_async_copy(xo_sc.at[pl.ds(S + r0, TQ), :], out_hbm.at[0, pl.ds(r0, TQ), :],
                                     sems.at[out_sem + t])

    order = [c_cp, x_cps[0]] + wma_cps + [wq_cps[0], k0_cp, v0_cp, wq_cps[1], wr_cp,
                                           x_cps[1], wq_cps[2], wo_cps[0], k_cp, v_cp]
    for t in range(1, NWC):
        order += [wq_cps[t + 2]] if t + 2 < NWC else []
        order += [wo_cps[t]]
    for cp in order + wmb_cps + x_cps[2:] + ffn_cps:
        cp.start()

    c_cp.wait()
    cf = c_sc[...].astype(F32)
    c16 = jnp.broadcast_to((cf * jax.nn.sigmoid(cf)).astype(BF), (16, D))

    def mod_cols(c0, n):
        mod_sc[:, c0:c0 + n] = _dot(c16, wmod_sc[:, c0:c0 + n])[0:8, :]

    def mod(i):
        return mod_sc[0:1, i * D:(i + 1) * D]

    x_cps[0].wait()
    xc0, rstd0 = _normalize(x_sc[0:TQ, :].astype(F32))
    xh0 = xc0 * rstd0
    for t in range(NMA):
        wma_cps[t].wait()
        mod_cols(t * MCA, MCA)
    h_sc[0:TQ // 2, :] = _pk((xh0 * (1.0 + mod(1)) + mod(0)).astype(BF))

    def q_proj(hslot, col, qslot):
        h = _ld(h_sc[pl.ds(_mult(hslot * (TQ // 2), TQ // 2), TQ // 2), :])
        q_sc[qslot] = (_dot(h, _ld(wq_sc[:, pl.ds(_mult(col, DH), DH)])) * QSCALE).astype(BF)

    wq_cps[0].wait()
    for m in range(DK):
        q_proj(0, m * DH, m)

    def ln1_piece(tile, k):
        xc, rstd = _normalize(x_sc[pl.ds(_mult(tile * TQ + k * RP, RP), RP), :].astype(F32))
        hslot = tile % 2 if isinstance(tile, int) else jnp.bitwise_and(tile, 1)
        h_sc[pl.ds(_mult(hslot * (TQ // 2) + k * (RP // 2), RP // 2), RP // 2), :] = _pk(
            (xc * rstd * (1.0 + mod(1)) + mod(0)).astype(BF))

    def epilogue_piece(tile, k, best):
        bval, bidx = best
        r0 = _mult(tile * TQ + k * RP, RP)
        att = att_sc[1, pl.ds(_mult(k * RP, RP), RP), :]
        xp = (x_sc[pl.ds(r0, RP), :].astype(F32) + mod(2) * att).astype(BF)
        xo_sc[pl.ds(r0, RP), :] = xp
        xf = xp.astype(F32)
        xc, rstd = _normalize(xf)
        xo_sc[pl.ds(S + r0, RP), :] = ((xf + ep_sc[1:2, :]) + (xc * rstd) * ep_sc[0:1, :]).astype(BF)
        r = jnp.sum(xc * ep_sc[2:3, :], axis=-1, keepdims=True) * rstd + ep_sc[3:4, 0:1]
        rows = r0 + lax.broadcasted_iota(jnp.int32, (RP, 1), 0)
        better = r > bval
        return jnp.where(better, r, bval), jnp.where(better, rows, bidx)

    def slot(j, g, b_hslot, b_col, o_wr, proj=None):
        if proj is not None:
            o_rd, wo_row, update = proj
            update(_dot(_ld(o_sc[:, o_rd * DH:(o_rd + DK) * DH]), _ld(wo_sc[pl.ds(_mult(_half(wo_row), DH // 2), WC // 2), 0:D])))
        s = lax.dot_general(q_sc[j % DK], k_sc[g], (((1,), (1,)), ((), ())), preferred_element_type=F32)
        q_proj(b_hslot, b_col, j % DK)
        p = jnp.exp2(s - jnp.max(s, axis=-1, keepdims=True))
        l = jnp.sum(p, axis=-1, keepdims=True)
        o = _dot(p.astype(BF), v_sc[g])
        rl = pltpu.reciprocal(l, approx=True)
        rl = rl * (2.0 - l * rl)
        o_sc[:, o_wr * DH:(o_wr + 1) * DH] = _pk((o * rl).astype(BF))

    def accumulate(d):
        acc_sc[...] += d

    def restart_unless(keep):
        def update(d):
            acc_sc[...] = jnp.where(keep, acc_sc[...], 0.0) + d
        return update

    k0_cp.wait()
    v0_cp.wait()
    wq_cps[1].wait()
    for j in range(DK):
        slot(j, 0, 0, WC + j * DH, 4 + j)

    def tile0_chunk(t, carry):
        @pl.when(t + 1 < NWC)
        def _():
            wait_like(cols(wq_hbm, 0, WC), cols(wq_sc.bitcast(BF), 0, WC), wq_sem + t + 1)
        wait_like(wo_hbm.at[pl.ds(0, WC), :], wo_sc.bitcast(BF).at[pl.ds(0, WC), pl.ds(0, D)], wo_sem + t - 1)

        @pl.when(t == 1)
        def _():
            x_cps[1].wait()

        @pl.when(t == 2)
        def _():
            k_cp.wait()
            v_cp.wait()
        last = t == NWC - 1
        col = t * WC
        b_col = jnp.where(last, 0, col + WC)
        b_hslot = last.astype(jnp.int32)
        g = lax.shift_right_logical(t, 1)
        for j in range(DK):
            proj = (4, col - WC, restart_unless(t > 1)) if j == 0 else None
            slot(j, g, b_hslot, b_col + j * DH, 4 + j, proj)
            if j < 3:
                ln1_piece(1, jnp.minimum(3 * (t - 1) + j, NP - 1))
        return carry

    lax.fori_loop(1, NWC, tile0_chunk, 0)
    wo_cps[NWC - 1].wait()

    for cp in wmb_cps:
        cp.wait()
    wr_cp.wait()
    for t in range(4):
        mod_cols(2048 + t * 1024, 1024)
    wr = wr_sc[...].astype(F32).reshape(1, D)
    cb1 = 1.0 + mod(4)
    ep_sc[0:1, :] = mod(5) * cb1
    ep_sc[1:2, :] = mod(5) * mod(3)
    ep_sc[2:3, :] = cb1 * wr
    ep_sc[3:4, :] = jnp.broadcast_to(jnp.sum(mod(3) * wr, axis=-1, keepdims=True), (1, D))

    ln1_slot = {(k * (NSL - DK)) // PPI: k for k in range(PPI)}
    epi_slot = {1 + k: (2 * k, 2 * k + 1) for k in range(PPI // 2)}

    def main_body(it, best):
        tile = lax.shift_right_logical(it, 1)
        part = jnp.bitwise_and(it, 1)
        first = part == 0

        @pl.when(first)
        def _():
            @pl.when(tile + 1 < NT)
            def _():
                wait_like(x_hbm.at[0, pl.ds(0, TQ), :], x_sc.at[pl.ds(0, TQ), :], x_sem + tile + 1)

            @pl.when(tile >= 2)
            def _():
                out_cp(tile - 2).start()

        base = part * (NSL * DH)
        nbase = NSL * DH - base
        hs_same = jnp.bitwise_and(tile, 1)
        hs_next = jnp.bitwise_and(tile + part, 1)

        def finish(d):
            t = acc_sc[...] + d
            att_sc[1 - part] = t
            acc_sc[...] = t

        for j in range(NSL):
            if j == 0:
                proj = (4, (HQ - DK) * DH - base, finish)
            elif j % DK == 0:
                update = restart_unless(jnp.logical_not(first)) if j == DK else accumulate
                proj = ((j - DK) % 8, base + (j - DK) * DH, update)
            else:
                proj = None
            if j + DK < NSL:
                b_hslot, b_col = hs_same, base + (j + DK) * DH
            else:
                b_hslot, b_col = hs_next, nbase + (j + DK - NSL) * DH
            slot(j, (NSL // REP) * part + j // REP, b_hslot, b_col, j % 8, proj)
            if j in ln1_slot:
                ln1_piece(jnp.minimum(tile + 1, NT - 1), part * PPI + ln1_slot[j])
            for k in epi_slot.get(j, ()):
                best = epilogue_piece(tile - 1, part * PPI + k, best)
        return best

    best = (jnp.full((RP, 1), -jnp.inf, F32), jnp.zeros((RP, 1), jnp.int32))
    best = lax.fori_loop(2, 2 * NT, main_body, best)

    out_cp(NT - 2).start()
    HT = TQ // LASTSPLIT
    for b in range(LASTSPLIT):
        rows = slice(b * HT, (b + 1) * HT)
        att_sc[1, rows, :] = acc_sc[rows, :] + _dot(_ld(o_sc[b * HT // 2:(b + 1) * HT // 2, 4 * DH:8 * DH]), _ld(wo_sc[(HQ - DK) * DH // 2:HQ * DH // 2, 0:D]))
    for k in range(NP):
        best = epilogue_piece(NT - 1, k, best)
    out_cp(NT - 1).start()

    bval, bidx = best
    idx = jnp.min(jnp.where(bval == jnp.max(bval, axis=0, keepdims=True), bidx, S))
    r0 = pl.multiple_of((idx // RP) * RP, RP)
    xf = xo_sc[pl.ds(r0, RP), :].astype(F32)
    xc, rstd = _normalize(xf)
    h2 = xc * rstd * cb1 + mod(3)
    r = jnp.sum(h2 * wr, axis=-1, keepdims=True)
    for cp in ffn_cps:
        cp.wait()
    h2b = h2.astype(BF)
    gate = _dot(h2b, wg_sc[...])
    up = _dot(h2b, wu_sc[...])
    act = (gate * jax.nn.sigmoid(gate) * up).astype(BF)
    y = _dot(act, wd_sc[:, 0:D]) * jax.nn.sigmoid(r)
    rows = r0 + lax.broadcasted_iota(jnp.int32, (RP, 1), 0)
    h_sc[0:RP // 2, :] = _pk((xf + mod(5) * (h2 + jnp.where(rows == idx, y, 0.0))).astype(BF))
    for t in range(NT):
        out_cp(t).wait()
    fix_cp = pltpu.make_async_copy(h_sc.bitcast(BF).at[pl.ds(0, RP), :], out_hbm.at[0, pl.ds(r0, RP), :], sems.at[out_sem + NT])
    fix_cp.start()
    fix_cp.wait()


@jax.jit
def pallas_adaLN_cond__sliding_block_cached__moe_arch_mod__prompt_kernel(
    A_x: jax.Array,
    A_k_cache: jax.Array,
    A_v_cache: jax.Array,
    A_wq: jax.Array,
    A_wo: jax.Array,
    B_x: jax.Array,
    B_w_r: jax.Array,
    B_w_gate: jax.Array,
    B_w_up: jax.Array,
    B_w_down: jax.Array,
    c: jax.Array,
    w_mod: jax.Array,
):
    del B_x
    any_spec = pl.BlockSpec(memory_space=pl.ANY)
    scratch = [
        pltpu.VMEM((TQ, D), jnp.uint32),
        pltpu.VMEM((DK, TQ, DH), BF),
        pltpu.VMEM((TQ // 2, 2 * WC), jnp.uint32),
        pltpu.VMEM((TQ, D), F32),
        pltpu.VMEM((2, TQ, D), F32),
        pltpu.VMEM((HKV, W, DH), BF),
        pltpu.VMEM((HKV, W, DH), BF),
        pltpu.VMEM((D // 2, HQ * DH + PAD), jnp.uint32),
        pltpu.VMEM((HQ * DH // 2, D + PAD), jnp.uint32),
        pltpu.VMEM((S, D), BF),
        pltpu.VMEM((2 * S, D), BF),
        pltpu.VMEM((D, 6 * D + PAD), BF),
        pltpu.VMEM((D, FF), BF),
        pltpu.VMEM((D, FF), BF),
        pltpu.VMEM((FF, D + PAD), BF),
        pltpu.VMEM((8, 6 * D), F32),
        pltpu.VMEM((8, D), F32),
        pltpu.VMEM((1, D), BF),
        pltpu.VMEM((D,), BF),
        pltpu.SemaphoreType.DMA((NSEM,)),
    ]
    return pl.pallas_call(
        _kernel,
        out_shape=jax.ShapeDtypeStruct(A_x.shape, A_x.dtype),
        in_specs=[any_spec] * 11,
        out_specs=any_spec,
        scratch_shapes=scratch,
        compiler_params=pltpu.CompilerParams(vmem_limit_bytes=100 * 1024 * 1024),
    )(A_x, A_k_cache, A_v_cache, A_wq, A_wo, B_w_r, B_w_gate, B_w_up, B_w_down, c, w_mod)
```

```python
import jax
import jax.numpy as jnp
from jax import lax
import jax.experimental.pallas as pl
import jax.experimental.pallas.tpu as pltpu

BF = jnp.bfloat16
F32 = jnp.float32

S, D = 2048, 1024
HQ, HKV, DH = 32, 4, 128
REP = HQ // HKV
W = 512
FF = 3584
EPS = 1e-5
QSCALE = (DH ** -0.5) * 1.4426950408889634

TQ = 256
NT = S // TQ
DK = 4
NSL = 16
NWC = HQ // DK
WC = DK * DH
RP = 16
NP = TQ // RP
PPI = NP // 2
PAD = 128
NMA, NMB = 4, 4
LASTSPLIT = 4
NSEM = 2 + NT + NMA + NMB + 2 * NWC + 4 + 3 + NT + 1


def _dot(a, b):
    return jnp.dot(a, b, preferred_element_type=F32)


def _pk(v):
    return pltpu.bitcast(v, jnp.uint32)


def _ld(ref_value):
    return pltpu.bitcast(ref_value, BF)


def _half(v):
    return v // 2 if isinstance(v, int) else lax.shift_right_logical(v, 1)


def _normalize(xf):
    xc = xf - jnp.mean(xf, axis=-1, keepdims=True)
    return xc, lax.rsqrt(jnp.mean(xc * xc, axis=-1, keepdims=True) + EPS)


def _mult(v, m):
    return v if isinstance(v, int) else pl.multiple_of(v, m)


def _kernel(x_hbm, k_hbm, v_hbm, wq_hbm, wo_hbm, wr_hbm, wg_hbm, wu_hbm, wd_hbm, c_hbm, wmod_hbm,
            out_hbm,
            h_sc, q_sc, o_sc, acc_sc, att_sc, k_sc, v_sc, wq_sc, wo_sc, x_sc, xo_sc,
            wmod_sc, wg_sc, wu_sc, wd_sc, mod_sc, ep_sc, c_sc, wr_sc, sems):

    nsem = [0]

    def copy(src, dst):
        nsem[0] += 1
        return pltpu.make_async_copy(src, dst, sems.at[nsem[0] - 1])

    def wait_like(src, dst, sem_index):
        pltpu.make_async_copy(src, dst, sems.at[sem_index]).wait()

    def cols(ref, c0, n):
        return ref.at[:, pl.ds(c0, n)]

    kv0 = k_hbm.shape[2] - W
    MCA, MCB = 2048 // NMA, 4096 // NMB
    c_cp = copy(c_hbm, c_sc)
    wr_cp = copy(wr_hbm, wr_sc)
    x_sem = nsem[0]
    x_cps = [copy(x_hbm.at[0, pl.ds(t * TQ, TQ), :], x_sc.bitcast(BF).at[pl.ds(t * TQ, TQ), :]) for t in range(NT)]
    wma_cps = [copy(cols(wmod_hbm, t * MCA, MCA), cols(wmod_sc, t * MCA, MCA)) for t in range(NMA)]
    wmb_cps = [copy(cols(wmod_hbm, 2048 + t * MCB, MCB), cols(wmod_sc, 2048 + t * MCB, MCB)) for t in range(NMB)]
    wq_sem = nsem[0]
    wq_cps = [copy(cols(wq_hbm, t * WC, WC), cols(wq_sc.bitcast(BF), t * WC, WC)) for t in range(NWC)]
    wo_sem = nsem[0]
    wo_cps = [copy(wo_hbm.at[pl.ds(t * WC, WC), :], wo_sc.bitcast(BF).at[pl.ds(t * WC, WC), pl.ds(0, D)]) for t in range(NWC)]
    k0_cp = copy(k_hbm.at[0, 0, pl.ds(kv0, W), :], k_sc.bitcast(BF).at[0])
    v0_cp = copy(v_hbm.at[0, 0, pl.ds(kv0, W), :], v_sc.bitcast(BF).at[0])
    k_cp = copy(k_hbm.at[0, pl.ds(1, HKV - 1), pl.ds(kv0, W), :], k_sc.bitcast(BF).at[pl.ds(1, HKV - 1)])
    v_cp = copy(v_hbm.at[0, pl.ds(1, HKV - 1), pl.ds(kv0, W), :], v_sc.bitcast(BF).at[pl.ds(1, HKV - 1)])
    ffn_cps = [copy(wg_hbm, wg_sc), copy(wu_hbm, wu_sc), copy(wd_hbm, wd_sc.at[:, pl.ds(0, D)])]
    out_sem = nsem[0]

    def out_cp(t):
        r0 = _mult(t * TQ, TQ)
        return pltpu.make_async_copy(xo_sc.bitcast(BF).at[pl.ds(S + r0, TQ), :], out_hbm.at[0, pl.ds(r0, TQ), :],
                                     sems.at[out_sem + t])

    order = [c_cp, x_cps[0]] + wma_cps + [wq_cps[0], k0_cp, v0_cp, wq_cps[1], wr_cp,
                                           x_cps[1], wq_cps[2], wo_cps[0], k_cp, v_cp]
    for t in range(1, NWC):
        order += [wq_cps[t + 2]] if t + 2 < NWC else []
        order += [wo_cps[t]]
    for cp in order + wmb_cps + x_cps[2:] + ffn_cps:
        cp.start()

    c_cp.wait()
    cf = c_sc[...].astype(F32)
    c16 = jnp.broadcast_to((cf * jax.nn.sigmoid(cf)).astype(BF), (16, D))

    def mod_cols(c0, n):
        mod_sc[:, c0:c0 + n] = _dot(c16, wmod_sc[:, c0:c0 + n])[0:8, :]

    def mod(i):
        return mod_sc[0:1, i * D:(i + 1) * D]

    x_cps[0].wait()
    xc0, rstd0 = _normalize(_ld(x_sc[0:TQ // 2, :]).astype(F32))
    xh0 = xc0 * rstd0
    for t in range(NMA):
        wma_cps[t].wait()
        mod_cols(t * MCA, MCA)
    h_sc[0:TQ // 2, :] = _pk((xh0 * (1.0 + mod(1)) + mod(0)).astype(BF))

    def q_proj(hslot, col, qslot):
        h = _ld(h_sc[pl.ds(_mult(hslot * (TQ // 2), TQ // 2), TQ // 2), :])
        q_sc[qslot] = _pk((_dot(h, _ld(wq_sc[:, pl.ds(_mult(col, DH), DH)])) * QSCALE).astype(BF))

    wq_cps[0].wait()
    for m in range(DK):
        q_proj(0, m * DH, m)

    def ln1_piece(tile, k):
        xc, rstd = _normalize(_ld(x_sc[pl.ds(_mult(tile * (TQ // 2) + k * (RP // 2), RP // 2), RP // 2), :]).astype(F32))
        hslot = tile % 2 if isinstance(tile, int) else jnp.bitwise_and(tile, 1)
        h_sc[pl.ds(_mult(hslot * (TQ // 2) + k * (RP // 2), RP // 2), RP // 2), :] = _pk(
            (xc * rstd * (1.0 + mod(1)) + mod(0)).astype(BF))

    def epilogue_piece(tile, k, best):
        bval, bidx = best
        r0 = _mult(tile * TQ + k * RP, RP)
        att = att_sc[1, pl.ds(_mult(k * RP, RP), RP), :]
        rh = _mult(tile * (TQ // 2) + k * (RP // 2), RP // 2)
        xp = (_ld(x_sc[pl.ds(rh, RP // 2), :]).astype(F32) + mod(2) * att).astype(BF)
        xo_sc[pl.ds(rh, RP // 2), :] = _pk(xp)
        xf = xp.astype(F32)
        xc, rstd = _normalize(xf)
        xo_sc[pl.ds(S // 2 + rh, RP // 2), :] = _pk(((xf + ep_sc[1:2, :]) + (xc * rstd) * ep_sc[0:1, :]).astype(BF))
        r = jnp.sum(xc * ep_sc[2:3, :], axis=-1, keepdims=True) * rstd + ep_sc[3:4, 0:1]
        rows = r0 + lax.broadcasted_iota(jnp.int32, (RP, 1), 0)
        better = r > bval
        return jnp.where(better, r, bval), jnp.where(better, rows, bidx)

    def slot(j, g, b_hslot, b_col, o_wr, proj=None):
        if proj is not None:
            o_rd, wo_row, update = proj
            update(_dot(_ld(o_sc[:, o_rd * DH:(o_rd + DK) * DH]), _ld(wo_sc[pl.ds(_mult(_half(wo_row), DH // 2), WC // 2), 0:D])))
        s = lax.dot_general(_ld(q_sc[j % DK]), _ld(k_sc[g]), (((1,), (1,)), ((), ())), preferred_element_type=F32)
        q_proj(b_hslot, b_col, j % DK)
        p = jnp.exp2(s - jnp.max(s, axis=-1, keepdims=True))
        l = jnp.sum(p, axis=-1, keepdims=True)
        o = _dot(p.astype(BF), _ld(v_sc[g]))
        rl = pltpu.reciprocal(l, approx=True)
        rl = rl * (2.0 - l * rl)
        o_sc[:, o_wr * DH:(o_wr + 1) * DH] = _pk((o * rl).astype(BF))

    def accumulate(d):
        acc_sc[...] += d

    def restart_unless(keep):
        def update(d):
            acc_sc[...] = jnp.where(keep, acc_sc[...], 0.0) + d
        return update

    k0_cp.wait()
    v0_cp.wait()
    wq_cps[1].wait()
    for j in range(DK):
        slot(j, 0, 0, WC + j * DH, 4 + j)

    def tile0_chunk(t, carry):
        @pl.when(t + 1 < NWC)
        def _():
            wait_like(cols(wq_hbm, 0, WC), cols(wq_sc.bitcast(BF), 0, WC), wq_sem + t + 1)
        wait_like(wo_hbm.at[pl.ds(0, WC), :], wo_sc.bitcast(BF).at[pl.ds(0, WC), pl.ds(0, D)], wo_sem + t - 1)

        @pl.when(t == 1)
        def _():
            x_cps[1].wait()

        @pl.when(t == 2)
        def _():
            k_cp.wait()
            v_cp.wait()
        last = t == NWC - 1
        col = t * WC
        b_col = jnp.where(last, 0, col + WC)
        b_hslot = last.astype(jnp.int32)
        g = lax.shift_right_logical(t, 1)
        for j in range(DK):
            proj = (4, col - WC, restart_unless(t > 1)) if j == 0 else None
            slot(j, g, b_hslot, b_col + j * DH, 4 + j, proj)
            if j < 3:
                ln1_piece(1, jnp.minimum(3 * (t - 1) + j, NP - 1))
        return carry

    lax.fori_loop(1, NWC, tile0_chunk, 0)
    wo_cps[NWC - 1].wait()

    for cp in wmb_cps:
        cp.wait()
    wr_cp.wait()
    for t in range(4):
        mod_cols(2048 + t * 1024, 1024)
    wr = wr_sc[...].astype(F32).reshape(1, D)
    cb1 = 1.0 + mod(4)
    ep_sc[0:1, :] = mod(5) * cb1
    ep_sc[1:2, :] = mod(5) * mod(3)
    ep_sc[2:3, :] = cb1 * wr
    ep_sc[3:4, :] = jnp.broadcast_to(jnp.sum(mod(3) * wr, axis=-1, keepdims=True), (1, D))

    ln1_slot = {(k * (NSL - DK)) // PPI: k for k in range(PPI)}
    epi_slot = {1 + k: (2 * k, 2 * k + 1) for k in range(PPI // 2)}

    def main_body(it, best):
        tile = lax.shift_right_logical(it, 1)
        part = jnp.bitwise_and(it, 1)
        first = part == 0

        @pl.when(first)
        def _():
            @pl.when(tile + 1 < NT)
            def _():
                wait_like(x_hbm.at[0, pl.ds(0, TQ), :], x_sc.bitcast(BF).at[pl.ds(0, TQ), :], x_sem + tile + 1)

            @pl.when(tile >= 2)
            def _():
                out_cp(tile - 2).start()

        base = part * (NSL * DH)
        nbase = NSL * DH - base
        hs_same = jnp.bitwise_and(tile, 1)
        hs_next = jnp.bitwise_and(tile + part, 1)

        def finish(d):
            t = acc_sc[...] + d
            att_sc[1 - part] = t
            acc_sc[...] = t

        for j in range(NSL):
            if j == 0:
                proj = (4, (HQ - DK) * DH - base, finish)
            elif j % DK == 0:
                update = restart_unless(jnp.logical_not(first)) if j == DK else accumulate
                proj = ((j - DK) % 8, base + (j - DK) * DH, update)
            else:
                proj = None
            if j + DK < NSL:
                b_hslot, b_col = hs_same, base + (j + DK) * DH
            else:
                b_hslot, b_col = hs_next, nbase + (j + DK - NSL) * DH
            slot(j, (NSL // REP) * part + j // REP, b_hslot, b_col, j % 8, proj)
            if j in ln1_slot:
                ln1_piece(jnp.minimum(tile + 1, NT - 1), part * PPI + ln1_slot[j])
            for k in epi_slot.get(j, ()):
                best = epilogue_piece(tile - 1, part * PPI + k, best)
        return best

    best = (jnp.full((RP, 1), -jnp.inf, F32), jnp.zeros((RP, 1), jnp.int32))
    best = lax.fori_loop(2, 2 * NT, main_body, best)

    out_cp(NT - 2).start()
    HT = TQ // LASTSPLIT
    for b in range(LASTSPLIT):
        rows = slice(b * HT, (b + 1) * HT)
        att_sc[1, rows, :] = acc_sc[rows, :] + _dot(_ld(o_sc[b * HT // 2:(b + 1) * HT // 2, 4 * DH:8 * DH]), _ld(wo_sc[(HQ - DK) * DH // 2:HQ * DH // 2, 0:D]))
    for k in range(NP):
        best = epilogue_piece(NT - 1, k, best)
    out_cp(NT - 1).start()

    bval, bidx = best
    idx = jnp.min(jnp.where(bval == jnp.max(bval, axis=0, keepdims=True), bidx, S))
    r0 = pl.multiple_of((idx // RP) * RP, RP)
    xf = _ld(xo_sc[pl.ds(pl.multiple_of((idx // RP) * (RP // 2), RP // 2), RP // 2), :]).astype(F32)
    xc, rstd = _normalize(xf)
    h2 = xc * rstd * cb1 + mod(3)
    r = jnp.sum(h2 * wr, axis=-1, keepdims=True)
    for cp in ffn_cps:
        cp.wait()
    h2b = h2.astype(BF)
    gate = _dot(h2b, wg_sc[...])
    up = _dot(h2b, wu_sc[...])
    act = (gate * jax.nn.sigmoid(gate) * up).astype(BF)
    y = _dot(act, wd_sc[:, 0:D]) * jax.nn.sigmoid(r)
    rows = r0 + lax.broadcasted_iota(jnp.int32, (RP, 1), 0)
    h_sc[0:RP // 2, :] = _pk((xf + mod(5) * (h2 + jnp.where(rows == idx, y, 0.0))).astype(BF))
    for t in range(NT):
        out_cp(t).wait()
    fix_cp = pltpu.make_async_copy(h_sc.bitcast(BF).at[pl.ds(0, RP), :], out_hbm.at[0, pl.ds(r0, RP), :], sems.at[out_sem + NT])
    fix_cp.start()
    fix_cp.wait()


@jax.jit
def pallas_adaLN_cond__sliding_block_cached__moe_arch_mod__prompt_kernel(
    A_x: jax.Array,
    A_k_cache: jax.Array,
    A_v_cache: jax.Array,
    A_wq: jax.Array,
    A_wo: jax.Array,
    B_x: jax.Array,
    B_w_r: jax.Array,
    B_w_gate: jax.Array,
    B_w_up: jax.Array,
    B_w_down: jax.Array,
    c: jax.Array,
    w_mod: jax.Array,
):
    del B_x
    any_spec = pl.BlockSpec(memory_space=pl.ANY)
    scratch = [
        pltpu.VMEM((TQ, D), jnp.uint32),
        pltpu.VMEM((DK, TQ // 2, DH), jnp.uint32),
        pltpu.VMEM((TQ // 2, 2 * WC), jnp.uint32),
        pltpu.VMEM((TQ, D), F32),
        pltpu.VMEM((2, TQ, D), F32),
        pltpu.VMEM((HKV, W // 2, DH), jnp.uint32),
        pltpu.VMEM((HKV, W // 2, DH), jnp.uint32),
        pltpu.VMEM((D // 2, HQ * DH + PAD), jnp.uint32),
        pltpu.VMEM((HQ * DH // 2, D + PAD), jnp.uint32),
        pltpu.VMEM((S // 2, D), jnp.uint32),
        pltpu.VMEM((S, D), jnp.uint32),
        pltpu.VMEM((D, 6 * D + PAD), BF),
        pltpu.VMEM((D, FF), BF),
        pltpu.VMEM((D, FF), BF),
        pltpu.VMEM((FF, D + PAD), BF),
        pltpu.VMEM((8, 6 * D), F32),
        pltpu.VMEM((8, D), F32),
        pltpu.VMEM((1, D), BF),
        pltpu.VMEM((D,), BF),
        pltpu.SemaphoreType.DMA((NSEM,)),
    ]
    return pl.pallas_call(
        _kernel,
        out_shape=jax.ShapeDtypeStruct(A_x.shape, A_x.dtype),
        in_specs=[any_spec] * 11,
        out_specs=any_spec,
        scratch_shapes=scratch,
        compiler_params=pltpu.CompilerParams(vmem_limit_bytes=100 * 1024 * 1024),
    )(A_x, A_k_cache, A_v_cache, A_wq, A_wo, B_w_r, B_w_gate, B_w_up, B_w_down, c, w_mod)
```

```python
import jax
import jax.numpy as jnp
from jax import lax
import jax.experimental.pallas as pl
import jax.experimental.pallas.tpu as pltpu

BF = jnp.bfloat16
F32 = jnp.float32

S, D = 2048, 1024
HQ, HKV, DH = 32, 4, 128
REP = HQ // HKV
W = 512
FF = 3584
EPS = 1e-5
QSCALE = (DH ** -0.5) * 1.4426950408889634

TQ = 256
NT = S // TQ
DK = 4
NSL = 16
NWC = HQ // DK
WC = DK * DH
RP = 16
NP = TQ // RP
PPI = NP // 2
NMA, NMB = 4, 4
LASTSPLIT = 4
NSEM = 2 + NT + NMA + NMB + 2 * NWC + 4 + 3 + NT + 1


def _dot(a, b):
    return jnp.dot(a, b, preferred_element_type=F32)


def _pk(v):
    return pltpu.bitcast(v, jnp.uint32)


def _ld(ref_value):
    return pltpu.bitcast(ref_value, BF)


def _half(v):
    return v // 2 if isinstance(v, int) else lax.shift_right_logical(v, 1)


def _normalize(xf):
    xc = xf - jnp.mean(xf, axis=-1, keepdims=True)
    return xc, lax.rsqrt(jnp.mean(xc * xc, axis=-1, keepdims=True) + EPS)


def _mult(v, m):
    return v if isinstance(v, int) else pl.multiple_of(v, m)


def _kernel(x_hbm, k_hbm, v_hbm, wq_hbm, wo_hbm, wr_hbm, wg_hbm, wu_hbm, wd_hbm, c_hbm, wmod_hbm,
            out_hbm,
            h_sc, q_sc, o_sc, acc_sc, att_sc, k_sc, v_sc, wq_sc, wo_sc, x_sc, xo_sc,
            wmod_sc, wg_sc, wu_sc, wd_sc, mod_sc, ep_sc, c_sc, wr_sc, sems):

    nsem = [0]

    def copy(src, dst):
        nsem[0] += 1
        return pltpu.make_async_copy(src, dst, sems.at[nsem[0] - 1])

    def wait_like(src, dst, sem_index):
        pltpu.make_async_copy(src, dst, sems.at[sem_index]).wait()

    def cols(ref, c0, n):
        return ref.at[:, pl.ds(c0, n)]

    kv0 = k_hbm.shape[2] - W
    MCA, MCB = 2048 // NMA, 4096 // NMB
    c_cp = copy(c_hbm, c_sc)
    wr_cp = copy(wr_hbm, wr_sc)
    x_sem = nsem[0]
    x_cps = [copy(x_hbm.at[0, pl.ds(t * TQ, TQ), :], x_sc.bitcast(BF).at[pl.ds(t * TQ, TQ), :]) for t in range(NT)]
    wma_cps = [copy(cols(wmod_hbm, t * MCA, MCA), cols(wmod_sc.bitcast(BF), t * MCA, MCA)) for t in range(NMA)]
    wmb_cps = [copy(cols(wmod_hbm, 2048 + t * MCB, MCB), cols(wmod_sc.bitcast(BF), 2048 + t * MCB, MCB)) for t in range(NMB)]
    wq_sem = nsem[0]
    wq_cps = [copy(cols(wq_hbm, t * WC, WC), cols(wq_sc.bitcast(BF), t * WC, WC)) for t in range(NWC)]
    wo_sem = nsem[0]
    wo_cps = [copy(wo_hbm.at[pl.ds(t * WC, WC), :], wo_sc.bitcast(BF).at[pl.ds(t * WC, WC), :]) for t in range(NWC)]
    k0_cp = copy(k_hbm.at[0, 0, pl.ds(kv0, W), :], k_sc.bitcast(BF).at[0])
    v0_cp = copy(v_hbm.at[0, 0, pl.ds(kv0, W), :], v_sc.bitcast(BF).at[0])
    k_cp = copy(k_hbm.at[0, pl.ds(1, HKV - 1), pl.ds(kv0, W), :], k_sc.bitcast(BF).at[pl.ds(1, HKV - 1)])
    v_cp = copy(v_hbm.at[0, pl.ds(1, HKV - 1), pl.ds(kv0, W), :], v_sc.bitcast(BF).at[pl.ds(1, HKV - 1)])
    ffn_cps = [copy(wg_hbm, wg_sc.bitcast(BF)), copy(wu_hbm, wu_sc.bitcast(BF)),
               copy(wd_hbm, wd_sc.bitcast(BF))]
    out_sem = nsem[0]

    def out_cp(t):
        r0 = _mult(t * TQ, TQ)
        return pltpu.make_async_copy(xo_sc.bitcast(BF).at[pl.ds(S + r0, TQ), :], out_hbm.at[0, pl.ds(r0, TQ), :],
                                     sems.at[out_sem + t])

    order = [c_cp, x_cps[0]] + wma_cps + [wq_cps[0], k0_cp, v0_cp, wq_cps[1], wr_cp,
                                           x_cps[1], wq_cps[2], wo_cps[0], k_cp, v_cp]
    for t in range(1, NWC):
        order += [wq_cps[t + 2]] if t + 2 < NWC else []
        order += [wo_cps[t]]
    for cp in order + wmb_cps + x_cps[2:] + ffn_cps:
        cp.start()

    c_cp.wait()
    cf = c_sc[...].astype(F32)
    c16 = jnp.broadcast_to((cf * jax.nn.sigmoid(cf)).astype(BF), (16, D))

    def mod_cols(c0, n):
        mod_sc[:, c0:c0 + n] = _dot(c16, _ld(wmod_sc[:, c0:c0 + n]))[0:8, :]

    def mod(i):
        return mod_sc[0:1, i * D:(i + 1) * D]

    x_cps[0].wait()
    xc0, rstd0 = _normalize(_ld(x_sc[0:TQ // 2, :]).astype(F32))
    xh0 = xc0 * rstd0
    for t in range(NMA):
        wma_cps[t].wait()
        mod_cols(t * MCA, MCA)
    h_sc[0:TQ // 2, :] = _pk((xh0 * (1.0 + mod(1)) + mod(0)).astype(BF))

    def q_proj(hslot, col, qslot):
        h = _ld(h_sc[pl.ds(_mult(hslot * (TQ // 2), TQ // 2), TQ // 2), :])
        q_sc[qslot] = _pk((_dot(h, _ld(wq_sc[:, pl.ds(_mult(col, DH), DH)])) * QSCALE).astype(BF))

    wq_cps[0].wait()
    for m in range(DK):
        q_proj(0, m * DH, m)

    def ln1_piece(tile, k):
        xc, rstd = _normalize(_ld(x_sc[pl.ds(_mult(tile * (TQ // 2) + k * (RP // 2), RP // 2), RP // 2), :]).astype(F32))
        hslot = tile % 2 if isinstance(tile, int) else jnp.bitwise_and(tile, 1)
        h_sc[pl.ds(_mult(hslot * (TQ // 2) + k * (RP // 2), RP // 2), RP // 2), :] = _pk(
            (xc * rstd * (1.0 + mod(1)) + mod(0)).astype(BF))

    def epilogue_piece(tile, k, best):
        bval, bidx = best
        r0 = _mult(tile * TQ + k * RP, RP)
        att = att_sc[1, pl.ds(_mult(k * RP, RP), RP), :]
        rh = _mult(tile * (TQ // 2) + k * (RP // 2), RP // 2)
        xp = (_ld(x_sc[pl.ds(rh, RP // 2), :]).astype(F32) + mod(2) * att).astype(BF)
        xo_sc[pl.ds(rh, RP // 2), :] = _pk(xp)
        xf = xp.astype(F32)
        xc, rstd = _normalize(xf)
        xo_sc[pl.ds(S // 2 + rh, RP // 2), :] = _pk(((xf + ep_sc[1:2, :]) + (xc * rstd) * ep_sc[0:1, :]).astype(BF))
        r = jnp.sum(xc * ep_sc[2:3, :], axis=-1, keepdims=True) * rstd + ep_sc[3:4, 0:1]
        rows = r0 + lax.broadcasted_iota(jnp.int32, (RP, 1), 0)
        better = r > bval
        return jnp.where(better, r, bval), jnp.where(better, rows, bidx)

    def slot(j, g, b_hslot, b_col, o_wr, proj=None):
        if proj is not None:
            o_rd, wo_row, update = proj
            update(_dot(_ld(o_sc[:, o_rd * DH:(o_rd + DK) * DH]), _ld(wo_sc[pl.ds(_mult(_half(wo_row), DH // 2), WC // 2), :])))
        s = lax.dot_general(_ld(q_sc[j % DK]), _ld(k_sc[g]), (((1,), (1,)), ((), ())), preferred_element_type=F32)
        q_proj(b_hslot, b_col, j % DK)
        p = jnp.exp2(s - jnp.max(s, axis=-1, keepdims=True))
        l = jnp.sum(p, axis=-1, keepdims=True)
        o = _dot(p.astype(BF), _ld(v_sc[g]))
        rl = pltpu.reciprocal(l, approx=True)
        rl = rl * (2.0 - l * rl)
        o_sc[:, o_wr * DH:(o_wr + 1) * DH] = _pk((o * rl).astype(BF))

    def accumulate(d):
        acc_sc[...] += d

    def restart_unless(keep):
        def update(d):
            acc_sc[...] = jnp.where(keep, acc_sc[...], 0.0) + d
        return update

    k0_cp.wait()
    v0_cp.wait()
    wq_cps[1].wait()
    for j in range(DK):
        slot(j, 0, 0, WC + j * DH, 4 + j)

    def tile0_chunk(t, carry):
        @pl.when(t + 1 < NWC)
        def _():
            wait_like(cols(wq_hbm, 0, WC), cols(wq_sc.bitcast(BF), 0, WC), wq_sem + t + 1)
        wait_like(wo_hbm.at[pl.ds(0, WC), :], wo_sc.bitcast(BF).at[pl.ds(0, WC), :], wo_sem + t - 1)

        @pl.when(t == 1)
        def _():
            x_cps[1].wait()

        @pl.when(t == 2)
        def _():
            k_cp.wait()
            v_cp.wait()
        last = t == NWC - 1
        col = t * WC
        b_col = jnp.where(last, 0, col + WC)
        b_hslot = last.astype(jnp.int32)
        g = lax.shift_right_logical(t, 1)
        for j in range(DK):
            proj = (4, col - WC, restart_unless(t > 1)) if j == 0 else None
            slot(j, g, b_hslot, b_col + j * DH, 4 + j, proj)
            if j < 3:
                ln1_piece(1, jnp.minimum(3 * (t - 1) + j, NP - 1))
        return carry

    lax.fori_loop(1, NWC, tile0_chunk, 0)
    wo_cps[NWC - 1].wait()

    for cp in wmb_cps:
        cp.wait()
    wr_cp.wait()
    for t in range(4):
        mod_cols(2048 + t * 1024, 1024)
    wr = wr_sc[...].astype(F32).reshape(1, D)
    cb1 = 1.0 + mod(4)
    ep_sc[0:1, :] = mod(5) * cb1
    ep_sc[1:2, :] = mod(5) * mod(3)
    ep_sc[2:3, :] = cb1 * wr
    ep_sc[3:4, :] = jnp.broadcast_to(jnp.sum(mod(3) * wr, axis=-1, keepdims=True), (1, D))

    ln1_slot = {(k * (NSL - DK)) // PPI: k for k in range(PPI)}
    epi_slot = {1 + k: (2 * k, 2 * k + 1) for k in range(PPI // 2)}

    def main_body(it, best):
        tile = lax.shift_right_logical(it, 1)
        part = jnp.bitwise_and(it, 1)
        first = part == 0

        @pl.when(first)
        def _():
            @pl.when(tile + 1 < NT)
            def _():
                wait_like(x_hbm.at[0, pl.ds(0, TQ), :], x_sc.bitcast(BF).at[pl.ds(0, TQ), :], x_sem + tile + 1)

            @pl.when(tile >= 2)
            def _():
                out_cp(tile - 2).start()

        base = part * (NSL * DH)
        nbase = NSL * DH - base
        hs_same = jnp.bitwise_and(tile, 1)
        hs_next = jnp.bitwise_and(tile + part, 1)

        def finish(d):
            t = acc_sc[...] + d
            att_sc[1 - part] = t
            acc_sc[...] = t

        for j in range(NSL):
            if j == 0:
                proj = (4, (HQ - DK) * DH - base, finish)
            elif j % DK == 0:
                update = restart_unless(jnp.logical_not(first)) if j == DK else accumulate
                proj = ((j - DK) % 8, base + (j - DK) * DH, update)
            else:
                proj = None
            if j + DK < NSL:
                b_hslot, b_col = hs_same, base + (j + DK) * DH
            else:
                b_hslot, b_col = hs_next, nbase + (j + DK - NSL) * DH
            slot(j, (NSL // REP) * part + j // REP, b_hslot, b_col, j % 8, proj)
            if j in ln1_slot:
                ln1_piece(jnp.minimum(tile + 1, NT - 1), part * PPI + ln1_slot[j])
            for k in epi_slot.get(j, ()):
                best = epilogue_piece(tile - 1, part * PPI + k, best)
        return best

    best = (jnp.full((RP, 1), -jnp.inf, F32), jnp.zeros((RP, 1), jnp.int32))
    best = lax.fori_loop(2, 2 * NT, main_body, best)

    out_cp(NT - 2).start()
    HT = TQ // LASTSPLIT
    for b in range(LASTSPLIT):
        rows = slice(b * HT, (b + 1) * HT)
        att_sc[1, rows, :] = acc_sc[rows, :] + _dot(_ld(o_sc[b * HT // 2:(b + 1) * HT // 2, 4 * DH:8 * DH]), _ld(wo_sc[(HQ - DK) * DH // 2:HQ * DH // 2, :]))
    for k in range(NP):
        best = epilogue_piece(NT - 1, k, best)
    out_cp(NT - 1).start()

    bval, bidx = best
    idx = jnp.min(jnp.where(bval == jnp.max(bval, axis=0, keepdims=True), bidx, S))
    r0 = pl.multiple_of((idx // RP) * RP, RP)
    xf = _ld(xo_sc[pl.ds(pl.multiple_of((idx // RP) * (RP // 2), RP // 2), RP // 2), :]).astype(F32)
    xc, rstd = _normalize(xf)
    h2 = xc * rstd * cb1 + mod(3)
    r = jnp.sum(h2 * wr, axis=-1, keepdims=True)
    for cp in ffn_cps:
        cp.wait()
    h2b = h2.astype(BF)
    gate = _dot(h2b, _ld(wg_sc[...]))
    up = _dot(h2b, _ld(wu_sc[...]))
    act = (gate * jax.nn.sigmoid(gate) * up).astype(BF)
    y = _dot(act, _ld(wd_sc[...])) * jax.nn.sigmoid(r)
    rows = r0 + lax.broadcasted_iota(jnp.int32, (RP, 1), 0)
    h_sc[0:RP // 2, :] = _pk((xf + mod(5) * (h2 + jnp.where(rows == idx, y, 0.0))).astype(BF))
    for t in range(NT):
        out_cp(t).wait()
    fix_cp = pltpu.make_async_copy(h_sc.bitcast(BF).at[pl.ds(0, RP), :], out_hbm.at[0, pl.ds(r0, RP), :], sems.at[out_sem + NT])
    fix_cp.start()
    fix_cp.wait()


@jax.jit
def pallas_adaLN_cond__sliding_block_cached__moe_arch_mod__prompt_kernel(
    A_x: jax.Array,
    A_k_cache: jax.Array,
    A_v_cache: jax.Array,
    A_wq: jax.Array,
    A_wo: jax.Array,
    B_x: jax.Array,
    B_w_r: jax.Array,
    B_w_gate: jax.Array,
    B_w_up: jax.Array,
    B_w_down: jax.Array,
    c: jax.Array,
    w_mod: jax.Array,
):
    del B_x
    any_spec = pl.BlockSpec(memory_space=pl.ANY)
    scratch = [
        pltpu.VMEM((TQ, D), jnp.uint32),
        pltpu.VMEM((DK, TQ // 2, DH), jnp.uint32),
        pltpu.VMEM((TQ // 2, 2 * WC), jnp.uint32),
        pltpu.VMEM((TQ, D), F32),
        pltpu.VMEM((2, TQ, D), F32),
        pltpu.VMEM((HKV, W // 2, DH), jnp.uint32),
        pltpu.VMEM((HKV, W // 2, DH), jnp.uint32),
        pltpu.VMEM((D // 2, HQ * DH), jnp.uint32),
        pltpu.VMEM((HQ * DH // 2, D), jnp.uint32),
        pltpu.VMEM((S // 2, D), jnp.uint32),
        pltpu.VMEM((S, D), jnp.uint32),
        pltpu.VMEM((D // 2, 6 * D), jnp.uint32),
        pltpu.VMEM((D // 2, FF), jnp.uint32),
        pltpu.VMEM((D // 2, FF), jnp.uint32),
        pltpu.VMEM((FF // 2, D), jnp.uint32),
        pltpu.VMEM((8, 6 * D), F32),
        pltpu.VMEM((8, D), F32),
        pltpu.VMEM((1, D), BF),
        pltpu.VMEM((D,), BF),
        pltpu.SemaphoreType.DMA((NSEM,)),
    ]
    return pl.pallas_call(
        _kernel,
        out_shape=jax.ShapeDtypeStruct(A_x.shape, A_x.dtype),
        in_specs=[any_spec] * 11,
        out_specs=any_spec,
        scratch_shapes=scratch,
        compiler_params=pltpu.CompilerParams(vmem_limit_bytes=100 * 1024 * 1024),
    )(A_x, A_k_cache, A_v_cache, A_wq, A_wo, B_w_r, B_w_gate, B_w_up, B_w_down, c, w_mod)
```

```python
import jax
import jax.numpy as jnp
from jax import lax
import jax.experimental.pallas as pl
import jax.experimental.pallas.tpu as pltpu

BF = jnp.bfloat16
F32 = jnp.float32

S, D = 2048, 1024
HQ, HKV, DH = 32, 4, 128
REP = HQ // HKV
W = 512
FF = 3584
EPS = 1e-5
QSCALE = (DH ** -0.5) * 1.4426950408889634

TQ = 256
NT = S // TQ
DK = 4
NSL = 16
NWC = HQ // DK
WC = DK * DH
RP = 16
NP = TQ // RP
PPI = NP // 2
PAD = 128
NMA, NMB = 4, 4
LASTSPLIT = 4
NSEM = 2 + NT + NMA + NMB + 2 * NWC + 4 + 3 + NT + 1


def _dot(a, b):
    return jnp.dot(a, b, preferred_element_type=F32)


def _pk(v):
    return pltpu.bitcast(v, jnp.uint32)


def _ld(ref_value):
    return pltpu.bitcast(ref_value, BF)


def _normalize(xf):
    xc = xf - jnp.mean(xf, axis=-1, keepdims=True)
    return xc, lax.rsqrt(jnp.mean(xc * xc, axis=-1, keepdims=True) + EPS)


def _mult(v, m):
    return v if isinstance(v, int) else pl.multiple_of(v, m)


def _kernel(x_hbm, k_hbm, v_hbm, wq_hbm, wo_hbm, wr_hbm, wg_hbm, wu_hbm, wd_hbm, c_hbm, wmod_hbm,
            out_hbm,
            h_sc, q_sc, o_sc, acc_sc, att_sc, k_sc, v_sc, wq_sc, wo_sc, x_sc, xp_sc, out_sc,
            wmod_sc, wg_sc, wu_sc, wd_sc, mod_sc, ep_sc, c_sc, wr_sc, sems):

    nsem = [0]

    def copy(src, dst):
        nsem[0] += 1
        return pltpu.make_async_copy(src, dst, sems.at[nsem[0] - 1])

    def wait_like(src, dst, sem_index):
        pltpu.make_async_copy(src, dst, sems.at[sem_index]).wait()

    def cols(ref, c0, n):
        return ref.at[:, pl.ds(c0, n)]

    kv0 = k_hbm.shape[2] - W
    MCA, MCB = 2048 // NMA, 4096 // NMB
    c_cp = copy(c_hbm, c_sc)
    wr_cp = copy(wr_hbm, wr_sc)
    x_sem = nsem[0]
    x_cps = [copy(x_hbm.at[0, pl.ds(t * TQ, TQ), :], x_sc.at[pl.ds(t * TQ, TQ), :]) for t in range(NT)]
    wma_cps = [copy(cols(wmod_hbm, t * MCA, MCA), cols(wmod_sc, t * MCA, MCA)) for t in range(NMA)]
    wmb_cps = [copy(cols(wmod_hbm, 2048 + t * MCB, MCB), cols(wmod_sc, 2048 + t * MCB, MCB)) for t in range(NMB)]
    wq_sem = nsem[0]
    wq_cps = [copy(cols(wq_hbm, t * WC, WC), cols(wq_sc, t * WC, WC)) for t in range(NWC)]
    wo_sem = nsem[0]
    wo_cps = [copy(wo_hbm.at[pl.ds(t * WC, WC), :], wo_sc.at[pl.ds(t * WC, WC), pl.ds(0, D)]) for t in range(NWC)]
    k0_cp = copy(k_hbm.at[0, 0, pl.ds(kv0, W), :], k_sc.at[0])
    v0_cp = copy(v_hbm.at[0, 0, pl.ds(kv0, W), :], v_sc.at[0])
    k_cp = copy(k_hbm.at[0, pl.ds(1, HKV - 1), pl.ds(kv0, W), :], k_sc.at[pl.ds(1, HKV - 1)])
    v_cp = copy(v_hbm.at[0, pl.ds(1, HKV - 1), pl.ds(kv0, W), :], v_sc.at[pl.ds(1, HKV - 1)])
    ffn_cps = [copy(wg_hbm, wg_sc), copy(wu_hbm, wu_sc), copy(wd_hbm, wd_sc.at[:, pl.ds(0, D)])]
    out_sem = nsem[0]

    def out_cp(t):
        r0 = _mult(t * TQ, TQ)
        return pltpu.make_async_copy(out_sc.at[pl.ds(r0, TQ), :], out_hbm.at[0, pl.ds(r0, TQ), :],
                                     sems.at[out_sem + t])

    order = [c_cp, x_cps[0]] + wma_cps + [wq_cps[0], k0_cp, v0_cp, wq_cps[1], wr_cp,
                                           x_cps[1], wq_cps[2], wo_cps[0], k_cp, v_cp]
    for t in range(1, NWC):
        order += [wq_cps[t + 2]] if t + 2 < NWC else []
        order += [wo_cps[t]]
    for cp in order + wmb_cps + x_cps[2:] + ffn_cps:
        cp.start()

    c_cp.wait()
    cf = c_sc[...].astype(F32)
    c16 = jnp.broadcast_to((cf * jax.nn.sigmoid(cf)).astype(BF), (16, D))

    def mod_cols(c0, n):
        mod_sc[:, c0:c0 + n] = _dot(c16, wmod_sc[:, c0:c0 + n])[0:8, :]

    def mod(i):
        return mod_sc[0:1, i * D:(i + 1) * D]

    x_cps[0].wait()
    xc0, rstd0 = _normalize(x_sc[0:TQ, :].astype(F32))
    xh0 = xc0 * rstd0
    for t in range(NMA):
        wma_cps[t].wait()
        mod_cols(t * MCA, MCA)
    h_sc[0:TQ // 2, :] = _pk((xh0 * (1.0 + mod(1)) + mod(0)).astype(BF))

    def q_proj(hslot, col, qslot):
        h = _ld(h_sc[pl.ds(_mult(hslot * (TQ // 2), TQ // 2), TQ // 2), :])
        q_sc[qslot] = _pk((_dot(h, wq_sc[:, pl.ds(_mult(col, DH), DH)]) * QSCALE).astype(BF))

    wq_cps[0].wait()
    for m in range(DK):
        q_proj(0, m * DH, m)

    def ln1_piece(tile, k):
        xc, rstd = _normalize(x_sc[pl.ds(_mult(tile * TQ + k * RP, RP), RP), :].astype(F32))
        hslot = tile % 2 if isinstance(tile, int) else jnp.bitwise_and(tile, 1)
        h_sc[pl.ds(_mult(hslot * (TQ // 2) + k * (RP // 2), RP // 2), RP // 2), :] = _pk(
            (xc * rstd * (1.0 + mod(1)) + mod(0)).astype(BF))

    def epilogue_piece(tile, k, best):
        bval, bidx = best
        r0 = _mult(tile * TQ + k * RP, RP)
        att = att_sc[1, pl.ds(_mult(k * RP, RP), RP), :]
        rh = _mult(tile * (TQ // 2) + k * (RP // 2), RP // 2)
        xp = (x_sc[pl.ds(r0, RP), :].astype(F32) + mod(2) * att).astype(BF)
        xp_sc[pl.ds(rh, RP // 2), :] = _pk(xp)
        xf = xp.astype(F32)
        xc, rstd = _normalize(xf)
        out_sc[pl.ds(r0, RP), :] = ((xf + ep_sc[1:2, :]) + (xc * rstd) * ep_sc[0:1, :]).astype(BF)
        r = jnp.sum(xc * ep_sc[2:3, :], axis=-1, keepdims=True) * rstd + ep_sc[3:4, 0:1]
        rows = r0 + lax.broadcasted_iota(jnp.int32, (RP, 1), 0)
        better = r > bval
        return jnp.where(better, r, bval), jnp.where(better, rows, bidx)

    def slot(j, g, b_hslot, b_col, o_wr, proj=None):
        if proj is not None:
            o_rd, wo_row, update = proj
            update(_dot(_ld(o_sc[:, o_rd * DH:(o_rd + DK) * DH]), wo_sc[pl.ds(_mult(wo_row, DH), WC), 0:D]))
        s = lax.dot_general(_ld(q_sc[j % DK]), k_sc[g], (((1,), (1,)), ((), ())), preferred_element_type=F32)
        q_proj(b_hslot, b_col, j % DK)
        p = jnp.exp2(s - jnp.max(s, axis=-1, keepdims=True))
        l = jnp.sum(p, axis=-1, keepdims=True)
        o = _dot(p.astype(BF), v_sc[g])
        rl = pltpu.reciprocal(l, approx=True)
        rl = rl * (2.0 - l * rl)
        o_sc[:, o_wr * DH:(o_wr + 1) * DH] = _pk((o * rl).astype(BF))

    def accumulate(d):
        acc_sc[...] += d

    def restart_unless(keep):
        def update(d):
            acc_sc[...] = jnp.where(keep, acc_sc[...], 0.0) + d
        return update

    k0_cp.wait()
    v0_cp.wait()
    wq_cps[1].wait()
    for j in range(DK):
        slot(j, 0, 0, WC + j * DH, 4 + j)

    def tile0_chunk(t, carry):
        @pl.when(t + 1 < NWC)
        def _():
            wait_like(cols(wq_hbm, 0, WC), cols(wq_sc, 0, WC), wq_sem + t + 1)
        wait_like(wo_hbm.at[pl.ds(0, WC), :], wo_sc.at[pl.ds(0, WC), pl.ds(0, D)], wo_sem + t - 1)

        @pl.when(t == 1)
        def _():
            x_cps[1].wait()

        @pl.when(t == 2)
        def _():
            k_cp.wait()
            v_cp.wait()
        last = t == NWC - 1
        col = t * WC
        b_col = jnp.where(last, 0, col + WC)
        b_hslot = last.astype(jnp.int32)
        g = lax.shift_right_logical(t, 1)
        for j in range(DK):
            proj = (4, col - WC, restart_unless(t > 1)) if j == 0 else None
            slot(j, g, b_hslot, b_col + j * DH, 4 + j, proj)
            if j < 3:
                ln1_piece(1, jnp.minimum(3 * (t - 1) + j, NP - 1))
        return carry

    lax.fori_loop(1, NWC, tile0_chunk, 0)
    wo_cps[NWC - 1].wait()

    for cp in wmb_cps:
        cp.wait()
    wr_cp.wait()
    for t in range(4):
        mod_cols(2048 + t * 1024, 1024)
    wr = wr_sc[...].astype(F32).reshape(1, D)
    cb1 = 1.0 + mod(4)
    ep_sc[0:1, :] = mod(5) * cb1
    ep_sc[1:2, :] = mod(5) * mod(3)
    ep_sc[2:3, :] = cb1 * wr
    ep_sc[3:4, :] = jnp.broadcast_to(jnp.sum(mod(3) * wr, axis=-1, keepdims=True), (1, D))

    ln1_slot = {(k * (NSL - DK)) // PPI: k for k in range(PPI)}
    epi_slot = {1 + k: (2 * k, 2 * k + 1) for k in range(PPI // 2)}

    def main_body(it, best):
        tile = lax.shift_right_logical(it, 1)
        part = jnp.bitwise_and(it, 1)
        first = part == 0

        @pl.when(first)
        def _():
            @pl.when(tile + 1 < NT)
            def _():
                wait_like(x_hbm.at[0, pl.ds(0, TQ), :], x_sc.at[pl.ds(0, TQ), :], x_sem + tile + 1)

            @pl.when(tile >= 2)
            def _():
                out_cp(tile - 2).start()

        base = part * (NSL * DH)
        nbase = NSL * DH - base
        hs_same = jnp.bitwise_and(tile, 1)
        hs_next = jnp.bitwise_and(tile + part, 1)

        def finish(d):
            t = acc_sc[...] + d
            att_sc[1 - part] = t
            acc_sc[...] = t

        for j in range(NSL):
            if j == 0:
                proj = (4, (HQ - DK) * DH - base, finish)
            elif j % DK == 0:
                update = restart_unless(jnp.logical_not(first)) if j == DK else accumulate
                proj = ((j - DK) % 8, base + (j - DK) * DH, update)
            else:
                proj = None
            if j + DK < NSL:
                b_hslot, b_col = hs_same, base + (j + DK) * DH
            else:
                b_hslot, b_col = hs_next, nbase + (j + DK - NSL) * DH
            slot(j, (NSL // REP) * part + j // REP, b_hslot, b_col, j % 8, proj)
            if j in ln1_slot:
                ln1_piece(jnp.minimum(tile + 1, NT - 1), part * PPI + ln1_slot[j])
            for k in epi_slot.get(j, ()):
                best = epilogue_piece(tile - 1, part * PPI + k, best)
        return best

    best = (jnp.full((RP, 1), -jnp.inf, F32), jnp.zeros((RP, 1), jnp.int32))
    best = lax.fori_loop(2, 2 * NT, main_body, best)

    out_cp(NT - 2).start()
    HT = TQ // LASTSPLIT
    for b in range(LASTSPLIT):
        rows = slice(b * HT, (b + 1) * HT)
        att_sc[1, rows, :] = acc_sc[rows, :] + _dot(_ld(o_sc[b * HT // 2:(b + 1) * HT // 2, 4 * DH:8 * DH]), wo_sc[(HQ - DK) * DH:HQ * DH, 0:D])
    for k in range(NP):
        best = epilogue_piece(NT - 1, k, best)
    out_cp(NT - 1).start()

    bval, bidx = best
    idx = jnp.min(jnp.where(bval == jnp.max(bval, axis=0, keepdims=True), bidx, S))
    r0 = pl.multiple_of((idx // RP) * RP, RP)
    xf = _ld(xp_sc[pl.ds(pl.multiple_of((idx // RP) * (RP // 2), RP // 2), RP // 2), :]).astype(F32)
    xc, rstd = _normalize(xf)
    h2 = xc * rstd * cb1 + mod(3)
    r = jnp.sum(h2 * wr, axis=-1, keepdims=True)
    for cp in ffn_cps:
        cp.wait()
    h2b = h2.astype(BF)
    gate = _dot(h2b, wg_sc[...])
    up = _dot(h2b, wu_sc[...])
    act = (gate * jax.nn.sigmoid(gate) * up).astype(BF)
    y = _dot(act, wd_sc[:, 0:D]) * jax.nn.sigmoid(r)
    rows = r0 + lax.broadcasted_iota(jnp.int32, (RP, 1), 0)
    fixed = (xf + mod(5) * (h2 + jnp.where(rows == idx, y, 0.0))).astype(BF)
    for t in range(NT):
        out_cp(t).wait()
    out_sc[pl.ds(r0, RP), :] = fixed
    fix_cp = pltpu.make_async_copy(out_sc.at[pl.ds(r0, RP), :], out_hbm.at[0, pl.ds(r0, RP), :],
                                   sems.at[out_sem + NT])
    fix_cp.start()
    fix_cp.wait()


@jax.jit
def pallas_adaLN_cond__sliding_block_cached__moe_arch_mod__prompt_kernel(
    A_x: jax.Array,
    A_k_cache: jax.Array,
    A_v_cache: jax.Array,
    A_wq: jax.Array,
    A_wo: jax.Array,
    B_x: jax.Array,
    B_w_r: jax.Array,
    B_w_gate: jax.Array,
    B_w_up: jax.Array,
    B_w_down: jax.Array,
    c: jax.Array,
    w_mod: jax.Array,
):
    del B_x
    any_spec = pl.BlockSpec(memory_space=pl.ANY)
    scratch = [
        pltpu.VMEM((TQ, D), jnp.uint32),
        pltpu.VMEM((DK, TQ // 2, DH), jnp.uint32),
        pltpu.VMEM((TQ // 2, 2 * WC), jnp.uint32),
        pltpu.VMEM((TQ, D), F32),
        pltpu.VMEM((2, TQ, D), F32),
        pltpu.VMEM((HKV, W, DH), BF),
        pltpu.VMEM((HKV, W, DH), BF),
        pltpu.VMEM((D, HQ * DH + PAD), BF),
        pltpu.VMEM((HQ * DH, D + PAD), BF),
        pltpu.VMEM((S, D), BF),
        pltpu.VMEM((S // 2, D), jnp.uint32),
        pltpu.VMEM((S, D), BF),
        pltpu.VMEM((D, 6 * D + PAD), BF),
        pltpu.VMEM((D, FF), BF),
        pltpu.VMEM((D, FF), BF),
        pltpu.VMEM((FF, D + PAD), BF),
        pltpu.VMEM((8, 6 * D), F32),
        pltpu.VMEM((8, D), F32),
        pltpu.VMEM((1, D), BF),
        pltpu.VMEM((D,), BF),
        pltpu.SemaphoreType.DMA((NSEM,)),
    ]
    return pl.pallas_call(
        _kernel,
        out_shape=jax.ShapeDtypeStruct(A_x.shape, A_x.dtype),
        in_specs=[any_spec] * 11,
        out_specs=any_spec,
        scratch_shapes=scratch,
        compiler_params=pltpu.CompilerParams(vmem_limit_bytes=100 * 1024 * 1024),
    )(A_x, A_k_cache, A_v_cache, A_wq, A_wo, B_w_r, B_w_gate, B_w_up, B_w_down, c, w_mod)
```
